```python
import jax
import jax.numpy as jnp

def _softmax(x, axis=-1):
    return jax.nn.softmax(x, axis=axis)

def _gelu(x):
    return jax.nn.gelu(x, approximate=True)

def _silu(x):
    return jax.nn.silu(x)

def _sigmoid(x):
    return jax.nn.sigmoid(x)

def _layernorm(x, axis=-1, eps=1e-05):
    m = jnp.mean(x, axis=axis, keepdims=True)
    v = jnp.var(x, axis=axis, keepdims=True)
    return (x - m) / jnp.sqrt(v + eps)

def _scatter_add(tgt, idx, src, axis=0):
    return tgt.at[idx].add(src)

def _segment_sum(src, seg, n):
    return jax.ops.segment_sum(src, seg, n)

class _Rng:

    def __init__(self, key):
        self._k = key

    def _next(self):
        self._k, sub = jax.random.split(self._k)
        return sub

    def normal(self, shape):
        return jax.random.normal(self._next(), shape, dtype=jnp.bfloat16)

    def randint(self, lo, hi, shape):
        return jax.random.randint(self._next(), shape, lo, hi, dtype=jnp.int32)

    def uniform(self, shape, lo=0.0, hi=1.0):
        return jax.random.uniform(self._next(), shape, jnp.bfloat16, lo, hi)

    def permutation(self, n):
        return jax.random.permutation(self._next(), n)
kernel_name = 'concat_heads__memory_aug_recurrent_mem_tr__spectral_gfnet__prompt'

def setup_inputs():
    _rng = _Rng(jax.random.key(int.from_bytes(__import__("os").urandom(4), "little")))
    _w = lambda a: (lambda t: t.astype(jnp.bfloat16) if jnp.issubdtype(t.dtype, jnp.floating) else t)(jnp.asarray(a))

    def _A_setup():
        B, S, Dm = (1, 2048, 1024)
        H, Dh = (32, 128)
        M, seg = (8, 32)
        seg = min(seg, S)
        S = S // seg * seg
        return {'x': _w((lambda *s: _rng.normal(s) * 0.05)(B, S, Dm)), 'mem0': _w((lambda *s: _rng.normal(s) * 0.05)(B, M, Dm)), 'Wq': _w((lambda *s: _rng.normal(s) * 0.05)(Dm, H, Dh) * Dm ** (-0.5)), 'Wk': _w((lambda *s: _rng.normal(s) * 0.05)(Dm, H, Dh) * Dm ** (-0.5)), 'Wv': _w((lambda *s: _rng.normal(s) * 0.05)(Dm, H, Dh) * Dm ** (-0.5)), 'Wo': _w((lambda *s: _rng.normal(s) * 0.05)(H, Dh, Dm) * (H * Dh) ** (-0.5)), 'seg_len': seg}
    _A_in = _A_setup()

    def _B_setup():
        B, S, D = (1, 2048, 1024)
        Df = D // 2 + 1
        return {'x': _w((lambda *s: _rng.normal(s) * 0.05)(B, S, D)), 'w_r': _w((lambda *s: _rng.normal(s) * 0.05)(S, Df) * 0.02), 'w_i': _w((lambda *s: _rng.normal(s) * 0.05)(S, Df) * 0.02)}
    _B_in = _B_setup()
    return {'A_x': _A_in['x'], 'A_mem0': _A_in['mem0'], 'A_Wq': _A_in['Wq'], 'A_Wk': _A_in['Wk'], 'A_Wv': _A_in['Wv'], 'A_Wo': _A_in['Wo'], 'A_seg_len': _A_in['seg_len'], 'B_x': _B_in['x'], 'B_w_r': _B_in['w_r'], 'B_w_i': _B_in['w_i']}

def reference(A_x, A_mem0, A_Wq, A_Wk, A_Wv, A_Wo, A_seg_len, B_x, B_w_r, B_w_i):

    def _A_ref(x, mem0, Wq, Wk, Wv, Wo, seg_len):
        B, S, Dm = x.shape
        H, Dh = (Wq.shape[1], Wq.shape[2])
        M = mem0.shape[1]
        scale = Dh ** (-0.5)
        n_seg = S // seg_len
        L = M + seg_len
        idx = jnp.arange(L)
        mask = (idx[:, None] < M) | (idx[:, None] >= idx[None, :])
        mem = mem0
        outs = []
        for s in range(n_seg):
            xs = x[:, s * seg_len:(s + 1) * seg_len, :].copy()
            h = jnp.concatenate([mem, xs], axis=1)
            q = jnp.einsum('btd,dhe->bhte', h, Wq)
            k = jnp.einsum('btd,dhe->bhte', h, Wk)
            v = jnp.einsum('btd,dhe->bhte', h, Wv)
            scores = jnp.einsum('bhqe,bhke->bhqk', q, k) * scale
            scores = jnp.where(mask[None, None], scores, -1000000000.0)
            p = _softmax(scores, axis=-1)
            o = jnp.einsum('bhqk,bhke->bhqe', p, v)
            o = jnp.einsum('bhte,hed->btd', o, Wo)
            mem = o[:, :M, :].copy()
            outs.append(o[:, M:, :])
        return jnp.concatenate(outs, axis=1)

    def _B_ref(x, w_r, w_i):
        B, S, D = x.shape
        X = (lambda x, axes=(-2, -1): jnp.fft.rfft2(x.astype(jnp.float32), axes=axes))(x, axes=(-2, -1))
        W = w_r + 1j * w_i
        X = X * W
        y = (lambda x, s, axes=(-2, -1): jnp.fft.irfft2(x, s=s, axes=axes).astype(jnp.bfloat16))(X, (S, D), axes=(-2, -1))
        return y
    a = _A_ref(A_x, A_mem0, A_Wq, A_Wk, A_Wv, A_Wo, A_seg_len)
    b = _B_ref(B_x, B_w_r, B_w_i)
    return jnp.concatenate([a, b], axis=-1)
```

```python
import functools

import jax
import jax.numpy as jnp
import numpy as np
from jax import lax
import jax.experimental.pallas as pl
import jax.experimental.pallas.tpu as pltpu

f32, bf16, u32 = jnp.float32, jnp.bfloat16, jnp.uint32

S, D = 2048, 1024
H, DH = 32, 128
M, SEG = 8, 32
L = M + SEG
NSEG = S // SEG
NT = 5
WC = NT * 128
OUT_CHUNK = 8


def _kd_of_column():
  kd = np.zeros(512, np.int64)
  l = np.arange(64)
  kd[0:64] = 8 * l
  kd[64:128] = 4 + 8 * l
  for t in (1, 2, 3):
    kd[128 * t:128 * t + 64] = t + 8 * l
    kd[128 * t + 64:128 * t + 128] = (8 - t) + 8 * l
  return kd


def _constants():
  kd = _kd_of_column()
  b = np.arange(128)
  sgn = (-1.0) ** b
  mf = np.zeros((4, 256, 256))
  mi = np.zeros((4, 256, 256))
  for t in range(4):
    k = kd[128 * t:128 * t + 128]
    e = np.exp(-2j * np.pi * np.outer(b, k) / D)
    c, s = e.real, e.imag
    lo = (np.arange(128) < 64)[None, :]
    if t == 0:
      mf[0, :128, :128] = np.where(lo, c, 0)
      mf[0, :128, 128:] = np.where(lo, s, 0)
      mf[0, 128:, :128] = np.where(lo, 0, c)
      mf[0, 128:, 128:] = np.where(lo, 0, s)
      mf[0, :128, 128] = sgn
      inv = 2.0 * mf[0].T
      inv[0, :] *= 0.5
      inv[128, :] *= 0.5
      mi[0] = inv
    else:
      sg = np.where(lo, 1.0, -1.0)
      mf[t, :128, :128] = c
      mf[t, :128, 128:] = s
      mf[t, 128:, :128] = sg * s
      mf[t, 128:, 128:] = -sg * c
      mi[t] = 2.0 * mf[t].T
  mi /= (S * D)
  perm = np.zeros((512, 512))
  perm[kd, np.arange(512)] = 1.0
  gf = np.zeros((16, 256, 128))
  gi = np.zeros((16, 256, 128))
  for k1 in range(16):
    g = np.exp(-2j * np.pi * np.outer(k1 + 16 * b, b) / S)
    gf[k1, :128], gf[k1, 128:] = g.real, g.imag
    gi[k1, :128], gi[k1, 128:] = g.real.T, -g.imag.T
  cast = lambda a: a.astype(np.float32).astype(jnp.bfloat16)
  return cast(mf), cast(mi), cast(perm), cast(gf), cast(gi)


def _dft4(z, sign):
  (ar, ai), (br, bi), (cr, ci), (dr, di) = z
  t0r, t0i, t1r, t1i = ar + cr, ai + ci, ar - cr, ai - ci
  t2r, t2i, t3r, t3i = br + dr, bi + di, br - dr, bi - di
  p = (t1r + t3i, t1i - t3r)
  m = (t1r - t3i, t1i + t3r)
  x1, x3 = (p, m) if sign < 0 else (m, p)
  return [(t0r + t2r, t0i + t2i), x1, (t0r - t2r, t0i - t2i), x3]


def _cmul_w16(z, n, sign):
  zr, zi = z
  if n == 0:
    return z
  if n == 4:
    return (zi, -zr) if sign < 0 else (-zi, zr)
  c = float(np.cos(2 * np.pi * n / 16))
  s = float(sign * np.sin(2 * np.pi * n / 16))
  if n == 2:
    return ((zr + zi) * c, (zi - zr) * c) if sign < 0 else ((zr - zi) * c, (zi + zr) * c)
  if n == 6:
    h = -c
    return ((zi - zr) * h, (zr + zi) * -h) if sign < 0 else ((zr + zi) * -h, (zr - zi) * h)
  return (zr * c - zi * s, zr * s + zi * c)


def _dft16(x, sign):
  t = [_dft4([x[a2], x[4 + a2], x[8 + a2], x[12 + a2]], sign) for a2 in range(4)]
  out = [None] * 16
  for k1 in range(4):
    r = _dft4([_cmul_w16(t[a2][k1], a2 * k1, sign) for a2 in range(4)], sign)
    for k2 in range(4):
      out[k1 + 4 * k2] = r[k2]
  return out


def _rnd(a):
  return a.astype(bf16).astype(f32)


def _dot(a, b):
  return jnp.dot(a, b, preferred_element_type=f32)


def _kernel(ax_h, mem_h, wq_h, wk_h, wv_h, wo_h, bx_h, wr_h, wi_h,
            mf_h, mi_h, pm_h, gf_h, gi_h, out_h,
            wqkv, wo, ax, mem0, bx, wf, mf, mi, pm, gf, gi, xs, ao,
            sem_in, sem_out):
  nsem = [0]

  def copy(src, dst):
    c = pltpu.make_async_copy(src, dst, sem_in.at[nsem[0]])
    nsem[0] += 1
    return c

  def group(pairs):
    i = nsem[0]
    nsem[0] += 1
    return [pltpu.make_async_copy(s, d, sem_in.at[i]) for s, d in pairs]

  RB = 256
  c_mf = copy(mf_h, mf)
  c_bx = [copy(bx_h.at[r * RB:(r + 1) * RB], bx.at[r * RB:(r + 1) * RB])
          for r in range(S // RB)]
  c_pm = copy(pm_h, pm)
  c_gf = copy(gf_h, gf)
  c_gi = copy(gi_h, gi)
  wr_u, wi_u = wr_h.bitcast(u32), wi_h.bitcast(u32)
  c_wf = [group([(wr_u.at[:, k, :], wf.at[k, 0]), (wi_u.at[:, k, :], wf.at[k, 1])])
          for k in range(8)]
  c_mi = copy(mi_h, mi)
  c_w = []
  for m, w_h in enumerate((wq_h, wk_h, wv_h)):
    w_u = w_h.bitcast(u32)
    c_w.append([group([(w_u.at[:, par, hp, :], wqkv.at[m, par, hp])
                       for hp in range(4 * g, 4 * g + 4) for par in range(2)])
                for g in range(4)])
  c_mem = copy(mem_h, mem0)
  c_ax0 = copy(ax_h.at[0:256], ax.at[0:256])
  c_wo = copy(wo_h.bitcast(u32), wo)
  c_ax1 = copy(ax_h.at[256:S], ax.at[256:S])

  c_mf.start()
  for c in c_bx:
    c.start()
  c_pm.start()
  c_gf.start()
  c_gi.start()
  for g in c_wf:
    for c in g:
      c.start()
  c_mi.start()
  for cm in c_w:
    for g in cm:
      for c in g:
        c.start()
  c_mem.start()
  c_ax0.start()
  c_wo.start()
  c_ax1.start()

  rc = float(np.sqrt(0.5))
  lane = lax.broadcasted_iota(jnp.int32, (128, 128), 1)

  def col(c):
    return pl.ds(c * 128, 128)

  with jax.named_scope("b_dfwd"):
    c_mf.wait()
    for r in range(S // RB):
      c_bx[r].wait()

      def dfwd(i, _):
        rows = pl.ds(pl.multiple_of(r * RB + i * 128, 128), 128)
        x = [bx[rows, col(a)].astype(f32) for a in range(8)]
        e0, e1, e2, e3 = x[0] + x[4], x[0] - x[4], x[2] + x[6], x[2] - x[6]
        o0, o1, o2, o3 = x[1] + x[5], x[1] - x[5], x[3] + x[7], x[3] - x[7]
        ep, op = e0 + e2, o0 + o2
        u, w = (o1 - o3) * rc, (o1 + o3) * rc
        z = [(ep + op, ep - op), (e1 + u, w + e3), (e0 - e2, o0 - o2), (e1 - u, w - e3)]
        for t in range(4):
          zz = jnp.concatenate(z[t], axis=1).astype(bf16)
          y = _dot(zz, mf[t])
          yr, yi = y[:, :128], y[:, 128:]
          if t == 0:
            xs[rows, col(4)] = jnp.where(lane == 0, yi, 0.0)
            xs[rows, col(NT + 4)] = jnp.zeros((128, 128), f32)
            yi = jnp.where(lane == 0, 0.0, yi)
          xs[rows, col(t)] = yr
          xs[rows, col(NT + t)] = yi
        return 0

      lax.fori_loop(0, RB // 128, dfwd, 0)

  def radix16(sign):
    def body(i, _):
      r0 = pl.multiple_of(i * 8, 8)
      for t in range(NT):
        x = [(xs[pl.ds(a * 128 + r0, 8), col(t)], xs[pl.ds(a * 128 + r0, 8), col(NT + t)])
             for a in range(16)]
        y = _dft16(x, sign)
        for a in range(16):
          xs[pl.ds(a * 128 + r0, 8), col(t)] = y[a][0]
          xs[pl.ds(a * 128 + r0, 8), col(NT + t)] = y[a][1]
      return 0
    lax.fori_loop(0, 16, body, 0)

  with jax.named_scope("b_r16f"):
    radix16(-1)

  with jax.named_scope("b_mid"):
    c_pm.wait()
    c_gf.wait()
    c_gi.wait()
    for g in c_wf:
      for c in g:
        c.wait()

    def cmat(g, v):
      t = _dot(g, v)
      return t[:128, :WC] - t[128:, WC:], t[128:, :WC] + t[:128, WC:]

    def mid(kp, _):
      for par in range(2):
        def half(w):
          return pltpu.bitcast(w << 16 if par == 0 else w & jnp.uint32(0xFFFF0000), f32)
        wm = jnp.concatenate([half(wf[kp, 0, :, 0:512]), half(wf[kp, 1, :, 0:512])], axis=0)
        wp = _dot(wm, pm[...])
        nr = jnp.broadcast_to(half(wf[kp, 0, :, 512:513]), (128, 128))
        ni = jnp.broadcast_to(half(wf[kp, 1, :, 512:513]), (128, 128))
        w_r = jnp.concatenate([wp[:128], nr], axis=1)
        w_i = jnp.concatenate([wp[128:], ni], axis=1)
        k1 = 2 * kp + par
        rows = pl.ds(pl.multiple_of(k1 * 128, 128), 128)
        yr, yi = cmat(gf[k1], xs[rows, :].astype(bf16))
        zr = yr * w_r - yi * w_i
        zi = yr * w_i + yi * w_r
        pr, pi = cmat(gi[k1], jnp.concatenate([zr, zi], axis=1).astype(bf16))
        xs[rows, 0:WC] = pr
        xs[rows, WC:2 * WC] = pi
      return 0

    lax.fori_loop(0, 8, mid, 0)

  with jax.named_scope("b_r16i"):
    radix16(1)

  with jax.named_scope("b_dinv"):
    c_mi.wait()

    def dinv(i, _):
      rows = pl.ds(pl.multiple_of(i * 128, 128), 128)
      z = []
      for t in range(4):
        ur, ui = xs[rows, col(t)], xs[rows, col(NT + t)]
        if t == 0:
          ui = jnp.where(lane == 0, xs[rows, col(4)], ui)
        y = _dot(jnp.concatenate([ur, ui], axis=1).astype(bf16), mi[t])
        z.append((y[:, :128], y[:, 128:]))
      (z0, z4), (p1, q1), (p2, q2), (p3, q3) = z
      ep, op = z0 + z4, z0 - z4
      e0, e2, o0, o2 = ep + p2, ep - p2, op + q2, op - q2
      e1, e3 = p1 + p3, q1 - q3
      u, w = (p1 - p3) * rc, (q1 + q3) * rc
      o1, o3 = w + u, w - u
      y = [e0 + e1, o0 + o1, e2 + e3, o2 + o3, e0 - e1, o0 - o1, e2 - e3, o2 - o3]
      for a in range(8):
        bx[rows, col(a)] = y[a].astype(bf16)
      return 0

    lax.fori_loop(0, S // 128, dinv, 0)

  c_ob = pltpu.make_async_copy(bx, out_h.at[:, D:2 * D], sem_out.at[0])
  c_ob.start()

  with jax.named_scope("relayout"):
    for m in range(3):
      for g in range(4):
        for c in c_w[m][g]:
          c.wait()

        def merge(hp, _):
          for r in range(4):
            rows = pl.ds(r * 128, 128)
            a, b = wqkv[m, 0, hp, rows, :], wqkv[m, 1, hp, rows, :]
            wqkv[m, 0, hp, rows, :] = (a & 0xFFFF) | (b << 16)
            wqkv[m, 1, hp, rows, :] = (a >> 16) | (b & jnp.uint32(0xFFFF0000))
          return 0

        lax.fori_loop(4 * g, 4 * g + 4, merge, 0)

  c_mem.wait()
  c_ax0.wait()
  c_wo.wait()
  c_ax1.wait()

  row = lax.broadcasted_iota(jnp.int32, (L, L), 0)
  colm = lax.broadcasted_iota(jnp.int32, (L, L), 1)
  mask = (row < M) | (row >= colm)
  scale = DH ** -0.5
  LA, LB, LC, G = 1, 3, 4, 4

  def w1(m, h):
    return pltpu.bitcast(wqkv[m, h % 2, h // 2], bf16)

  def w2(j, g):
    return pltpu.bitcast(wo[g * G * 64:(g + 1) * G * 64, j * 128:(j + 1) * 128], bf16)

  def out_copy(c):
    rows = pl.ds(pl.multiple_of(c * (OUT_CHUNK * SEG), OUT_CHUNK * SEG), OUT_CHUNK * SEG)
    return pltpu.make_async_copy(ao.at[rows], out_h.at[rows, 0:D], sem_out.at[1])

  def step(s, mem):
    rows = pl.ds(pl.multiple_of(s * SEG, SEG), SEG)
    hl = jnp.concatenate([mem, ax[rows, :].astype(f32)], axis=0)
    q, k, v, p, o = {}, {}, {}, {}, {}
    y = [None] * 8
    for i in range(H + LC):
      if i < H:
        q[i] = _dot(hl, w1(0, i))
        k[i] = _dot(hl, w1(1, i))
      h = i - LA
      if 0 <= h < H:
        sc = lax.dot_general(_rnd(q[h]), k[h].astype(bf16), (((1,), (1,)), ((), ())),
                             preferred_element_type=f32)
        sc = jnp.where(mask, sc * scale, -1e9)
        e = jnp.exp(sc - jnp.max(sc, axis=-1, keepdims=True))
        p[h] = e / jnp.sum(e, axis=-1, keepdims=True)
      if i < H:
        v[i] = _dot(hl, w1(2, i))
      h = i - LB
      if 0 <= h < H:
        o[h] = _rnd(_dot(_rnd(p[h]), v[h].astype(bf16)))
      h = i - LC
      if 0 <= h < H and h % G == G - 1:
        g = h // G
        og = jnp.concatenate([o[hh] for hh in range(g * G, g * G + G)], axis=1)
        for j in range(8):
          t = _dot(og, w2(j, g))
          y[j] = t if y[j] is None else y[j] + t
    yb = jnp.concatenate(y, axis=1).astype(bf16)
    ao[rows, :] = yb[M:]

    @pl.when(s % OUT_CHUNK == OUT_CHUNK - 1)
    def _():
      out_copy(s // OUT_CHUNK).start()

    return yb[:M].astype(f32)

  with jax.named_scope("a_loop"):
    lax.fori_loop(0, NSEG, step, mem0[...].astype(f32))

  c_ob.wait()
  for c in range(NSEG // OUT_CHUNK):
    out_copy(c).wait()


@functools.partial(jax.jit, static_argnames=("A_seg_len",))
def pallas_concat_heads__memory_aug_recurrent_mem_tr__spectral_gfnet__prompt_kernel(
    A_x, A_mem0, A_Wq, A_Wk, A_Wv, A_Wo, A_seg_len, B_x, B_w_r, B_w_i):
  assert A_seg_len == SEG and A_x.shape == (1, S, D) and A_Wq.shape == (D, H, DH)
  consts = _constants()
  hbm = pl.BlockSpec(memory_space=pl.ANY)
  out = pl.pallas_call(
      _kernel,
      out_shape=jax.ShapeDtypeStruct((S, 2 * D), bf16),
      in_specs=[hbm] * 14,
      out_specs=hbm,
      scratch_shapes=[
          pltpu.VMEM((3, 2, H // 2, D // 2, DH), u32),
          pltpu.VMEM((H * DH // 2, D), u32),
          pltpu.VMEM((S, D), bf16),
          pltpu.VMEM((M, D), bf16),
          pltpu.VMEM((S, D), bf16),
          pltpu.VMEM((8, 2, 128, D // 2 + 1), u32),
          pltpu.VMEM((4, 256, 256), bf16),
          pltpu.VMEM((4, 256, 256), bf16),
          pltpu.VMEM((512, 512), bf16),
          pltpu.VMEM((16, 256, 128), bf16),
          pltpu.VMEM((16, 256, 128), bf16),
          pltpu.VMEM((S, 2 * WC), f32),
          pltpu.VMEM((S, D), bf16),
          pltpu.SemaphoreType.DMA((48,)),
          pltpu.SemaphoreType.DMA((2,)),
      ],
      compiler_params=pltpu.CompilerParams(vmem_limit_bytes=110 * 2**20),
  )(A_x.reshape(S, D), A_mem0.reshape(M, D),
    A_Wq.reshape(D // 2, 2, H, DH), A_Wk.reshape(D // 2, 2, H, DH), A_Wv.reshape(D // 2, 2, H, DH),
    A_Wo.reshape(H * DH, D), B_x.reshape(S, D),
    B_w_r.reshape(128, 16, D // 2 + 1), B_w_i.reshape(128, 16, D // 2 + 1), *consts)
  return out.reshape(1, S, 2 * D)
```

```python
import functools

import jax
import jax.numpy as jnp
import numpy as np
from jax import lax
import jax.experimental.pallas as pl
import jax.experimental.pallas.tpu as pltpu

f32, bf16, u32 = jnp.float32, jnp.bfloat16, jnp.uint32

S, D = 2048, 1024
H, DH = 32, 128
M, SEG = 8, 32
L = M + SEG
NSEG = S // SEG
OUT_CHUNK = 8
G = 4
NG = H // G
PRE = 8
UNROLL = 3
KR = D // 2 + 8


def _kd_of_row():
  kd = np.zeros(512, np.int64)
  l = np.arange(64)
  for t in range(4):
    kd[128 * t:128 * t + 64] = t + 8 * l
    kd[128 * t + 64:128 * t + 128] = (8 - t if t else 4) + 8 * l
  return kd


def _spectrum_row_of_residue(r):
  if r < 4:
    return 128 * r
  return 64 if r == 4 else 128 * (8 - r) + 64


def _constants():
  kd = _kd_of_row()
  b = np.arange(128)
  lo = (b < 64)[:, None]
  md = np.zeros((4, 256, 256))
  for t in range(4):
    e = np.exp(-2j * np.pi * np.outer(kd[128 * t:128 * t + 128], b) / D)
    c, s = e.real, e.imag
    if t == 0:
      md[0, :128, :128], md[0, 128:, :128] = np.where(lo, c, 0), np.where(lo, s, 0)
      md[0, :128, 128:], md[0, 128:, 128:] = np.where(lo, 0, c), np.where(lo, 0, s)
      md[0, 128, :128] = (-1.0) ** b
    else:
      sg = np.where(lo, 1.0, -1.0)
      md[t, :128, :128], md[t, 128:, :128] = c, s
      md[t, :128, 128:], md[t, 128:, 128:] = sg * s, -sg * c
  pm = np.zeros((128, 128))
  pm[b, b // 16 + 8 * (b % 16)] = 1.0
  gs = np.zeros((16, 256, 128))
  for a in range(16):
    g = np.exp(-2j * np.pi * np.outer(a + 16 * b, b) / S)
    gs[a, :128], gs[a, 128:] = g.real, g.imag
  cast = lambda a: a.astype(np.float32).astype(jnp.bfloat16)
  return cast(md), cast(pm), cast(gs)


def _dft4(z, sign):
  (ar, ai), (br, bi), (cr, ci), (dr, di) = z
  t0r, t0i, t1r, t1i = ar + cr, ai + ci, ar - cr, ai - ci
  t2r, t2i, t3r, t3i = br + dr, bi + di, br - dr, bi - di
  p = (t1r + t3i, t1i - t3r)
  m = (t1r - t3i, t1i + t3r)
  x1, x3 = (p, m) if sign < 0 else (m, p)
  return [(t0r + t2r, t0i + t2i), x1, (t0r - t2r, t0i - t2i), x3]


def _cmul_w16(z, n, sign):
  zr, zi = z
  if n == 0:
    return z
  if n == 4:
    return (zi, -zr) if sign < 0 else (-zi, zr)
  c = float(np.cos(2 * np.pi * n / 16))
  s = float(sign * np.sin(2 * np.pi * n / 16))
  if n == 2:
    return ((zr + zi) * c, (zi - zr) * c) if sign < 0 else ((zr - zi) * c, (zi + zr) * c)
  if n == 6:
    h = -c
    return ((zi - zr) * h, (zr + zi) * -h) if sign < 0 else ((zr + zi) * -h, (zr - zi) * h)
  return (zr * c - zi * s, zr * s + zi * c)


def _dft16(x, sign):
  t = [_dft4([x[a2], x[4 + a2], x[8 + a2], x[12 + a2]], sign) for a2 in range(4)]
  out = [None] * 16
  for k1 in range(4):
    r = _dft4([_cmul_w16(t[a2][k1], a2 * k1, sign) for a2 in range(4)], sign)
    for k2 in range(4):
      out[k1 + 4 * k2] = r[k2]
  return out


def _rnd(a):
  return a.astype(bf16).astype(f32)


def _dot(a, b):
  return jnp.dot(a, b, preferred_element_type=f32)


def _dot_nt(a, b):
  return lax.dot_general(a, b, (((1,), (1,)), ((), ())), preferred_element_type=f32)


def _kernel(ax_h, mem_h, wq_h, wk_h, wv_h, wo_h, bx_h, wr_h, wi_h, md_h, pm_h, gs_h, out_h,
            wqkv, wo, ax, mem0, bx, wt, md, pm, gs, xs, wf, ao, xq, qp, sem_in, sem_out):
  nsem = [0]

  def group(pairs):
    i = nsem[0]
    nsem[0] += 1
    return [pltpu.make_async_copy(s, d, sem_in.at[i]) for s, d in pairs]

  def wait(copies):
    for c in copies:
      c.wait()

  bx_u = bx_h.bitcast(u32)
  c_const = group([(md_h, md), (pm_h, pm), (gs_h, gs)])
  c_bx = [group([(bx_u.at[:, a, :], bx.at[a])]) for a in range(8)]
  c_wt = [group([(w_h.at[:, a * 256:(a + 1) * 256], wt.at[i, :, a * 256:(a + 1) * 256])
                 for i, w_h in enumerate((wr_h, wi_h))]) for a in range(8)]
  w_u = [w_h.bitcast(u32) for w_h in (wq_h, wk_h, wv_h)]
  wo_u = wo_h.bitcast(u32)

  def w_group(m, g):
    return group([(w_u[m].at[:, par, hp, :], wqkv.at[m, par, hp])
                  for hp in range(G // 2 * g, G // 2 * (g + 1)) for par in range(2)])

  c_w = [[w_group(m, g) for g in range(NG)] for m in range(3)]
  c_wo = [group([(wo_u.at[g * G * 64:(g + 1) * G * 64], wo.at[g * G * 64:(g + 1) * G * 64])])
          for g in range(NG)]
  c_xq = group([(ax_h.at[:, SEG - PRE:SEG, :], xq)])
  c_a0 = group([(mem_h, mem0), (ax_h.at[0:1], ax.at[0:1])])
  c_a1 = group([(ax_h.at[1:NSEG], ax.at[1:NSEG])])

  def start(groups):
    for g in groups:
      for c in g:
        c.start()

  with jax.named_scope("dma_start"):
    start([c_const])
    for a in range(8):
      start([c_bx[a], c_wt[a]])
    start([c_xq] + c_w[0])

  rc = float(np.sqrt(0.5))

  def col(c):
    return pl.ds(c * 128, 128)

  def dcol(c):
    return pl.ds(pl.multiple_of(c * 128, 128), 128)

  with jax.named_scope("b_fwd"):
    wait(c_const)
    row8 = lax.broadcasted_iota(jnp.int32, (8, 128), 0)

    def fwd(ap, _):
      for a in range(8):
        @pl.when(ap == a)
        def _():
          wait(c_bx[a])
          wait(c_wt[a])
      for par in range(2):
        a = 2 * ap + par
        w = [bx[ap, :, col(j)] for j in range(8)]
        x = [pltpu.bitcast(v << 16 if par == 0 else v & jnp.uint32(0xFFFF0000), f32) for v in w]
        e0, e1, e2, e3 = x[0] + x[4], x[0] - x[4], x[2] + x[6], x[2] - x[6]
        o0, o1, o2, o3 = x[1] + x[5], x[1] - x[5], x[3] + x[7], x[3] - x[7]
        ep, op = e0 + e2, o0 + o2
        u, v = (o1 - o3) * rc, (o1 + o3) * rc
        z = [(ep + op, ep - op), (e1 + u, v + e3), (e0 - e2, o0 - o2), (e1 - u, v - e3)]
        tt = [_dot_nt(md[t], jnp.concatenate(z[t], axis=1).astype(bf16)) for t in range(4)]
        g = jnp.concatenate([gs[a, :128], gs[a, 128:]], axis=1)
        for t in range(4):
          r = _dot(tt[t].astype(bf16), g)
          rr, ri, ir, ii = r[:128, :128], r[:128, 128:], r[128:, :128], r[128:, 128:]
          if t == 0:
            xs[0, 512:KR, dcol(a)] = jnp.where(row8 == 0, ir[:8], 0.0)
            xs[1, 512:KR, dcol(a)] = jnp.where(row8 == 0, ii[:8], 0.0)
            ir = jnp.concatenate([jnp.where(row8 == 0, 0.0, ir[:8]), ir[8:]], axis=0)
            ii = jnp.concatenate([jnp.where(row8 == 0, 0.0, ii[:8]), ii[8:]], axis=0)
          xs[0, t * 128:(t + 1) * 128, dcol(a)] = rr - ii
          xs[1, t * 128:(t + 1) * 128, dcol(a)] = ri + ir
      cols = pl.ds(pl.multiple_of(ap * 256, 256), 256)
      for i in range(2):
        for tile in range(4):
          p = _dot(pm[...], wt[i, tile * 128:(tile + 1) * 128, cols]) * (2.0 / (S * D))
          for r in range(8):
            pr = p[16 * r:16 * r + 16]
            if tile == 0 and r == 0:
              first = lax.broadcasted_iota(jnp.int32, (16, 256), 0) == 0
              pr = jnp.where(first, pr * 0.5, pr)
            r0 = _spectrum_row_of_residue(r) + 16 * tile
            wf[i, r0:r0 + 16, cols] = pr
        ny = wt[i, 512:513, cols].astype(f32) * (1.0 / (S * D))
        wf[i, 512:KR, cols] = jnp.broadcast_to(ny, (8, 256))
      return 0

    lax.fori_loop(0, 8, fwd, 0)

  start([c_a0])
  for g in range(NG // 2):
    start([c_w[1][g], c_w[2][g], c_wo[g]])

  with jax.named_scope("b_mid"):
    def mid(i, _):
      rows = pl.ds(pl.multiple_of(i * 8, 8), 8)
      y = _dft16([(xs[0, rows, col(a)], xs[1, rows, col(a)]) for a in range(16)], -1)
      z = []
      for c in range(16):
        wr, wi = wf[0, rows, col(c)], wf[1, rows, col(c)]
        yr, yi = y[c]
        z.append((yr * wr - yi * wi, yr * wi + yi * wr))
      q = _dft16(z, 1)
      for a in range(16):
        xs[0, rows, col(a)] = q[a][0]
        xs[1, rows, col(a)] = q[a][1]
      return 0

    lax.fori_loop(0, KR // 8, mid, 0)

  bo_u = out_h.bitcast(u32)
  c_ob = [pltpu.make_async_copy(bx.at[a], bo_u.at[:, a, D:2 * D], sem_out.at[0])
          for a in range(8)]

  with jax.named_scope("b_inv"):
    lane = lax.broadcasted_iota(jnp.int32, (128, 128), 1)

    def inv(ap, _):
      ys = []
      for par in range(2):
        a = 2 * ap + par
        g = gs[a]
        rs = [_dot_nt(g, jnp.concatenate(
            [xs[0, t * 128:(t + 1) * 128, dcol(a)], xs[1, t * 128:(t + 1) * 128, dcol(a)]],
            axis=0).astype(bf16)) for t in range(4)]
        qn = jnp.concatenate([xs[0, 512:KR, dcol(a)], xs[1, 512:KR, dcol(a)]], axis=1)
        qn = jnp.concatenate([qn, jnp.zeros((120, 256), f32)], axis=0).astype(bf16)
        ny = _dot_nt(jnp.concatenate([g[:128], g[128:]], axis=1), qn)
        z = []
        for t in range(4):
          r = rs[t]
          ur = r[:128, :128] + r[128:, 128:]
          ui = r[:128, 128:] - r[128:, :128]
          if t == 0:
            ui = jnp.where(lane == 0, ny, ui)
          y = _dot(jnp.concatenate([ur, ui], axis=1).astype(bf16), md[t])
          z.append((y[:, :128], y[:, 128:]))
        (z0, z4), (p1, q1), (p2, q2), (p3, q3) = z
        ep, op = z0 + z4, z0 - z4
        e0, e2, o0, o2 = ep + p2, ep - p2, op + q2, op - q2
        e1, e3 = p1 + p3, q1 - q3
        u, v = (p1 - p3) * rc, (q1 + q3) * rc
        o1, o3 = v + u, v - u
        ys.append([e0 + e1, o0 + o1, e2 + e3, o2 + o3, e0 - e1, o0 - o1, e2 - e3, o2 - o3])
      for j in range(8):
        lo = pltpu.bitcast(_rnd(ys[0][j]), u32)
        hi = pltpu.bitcast(_rnd(ys[1][j]), u32)
        bx[ap, :, col(j)] = (lo >> 16) | hi
      return 0

    lax.fori_loop(0, 8, inv, 0)

  for g in range(NG // 2, NG):
    start([c_w[1][g], c_w[2][g], c_wo[g]])
  start([c_a1])

  def merge(m, hp):
    for r in range(4):
      rows = pl.ds(r * 128, 128)
      a, b = wqkv[m, 0, hp, rows, :], wqkv[m, 1, hp, rows, :]
      wqkv[m, 0, hp, rows, :] = (a & 0xFFFF) | (b << 16)
      wqkv[m, 1, hp, rows, :] = (a >> 16) | (b & jnp.uint32(0xFFFF0000))

  def w1(m, h):
    return pltpu.bitcast(wqkv[m, h % 2, h // 2], bf16)

  def w2(j, g):
    return pltpu.bitcast(wo[g * G * 64:(g + 1) * G * 64, j * 128:(j + 1) * 128], bf16)

  with jax.named_scope("q_pre"):
    wait(c_xq)
    for g in range(NG):
      wait(c_w[0][g])

      def q_pre(hp, _):
        merge(0, hp)
        xv = xq[...].reshape(NSEG * PRE, D)
        for par in range(2):
          qp[2 * hp + par] = _rnd(_dot(xv, pltpu.bitcast(wqkv[0, par, hp], bf16)))
        return 0

      lax.fori_loop(G // 2 * g, G // 2 * (g + 1), q_pre, 0)

  row = lax.broadcasted_iota(jnp.int32, (L, L), 0)
  colm = lax.broadcasted_iota(jnp.int32, (L, L), 1)
  mask = (row < M) | (row >= colm)
  scale = DH ** -0.5

  def out_copy(c):
    n = OUT_CHUNK * SEG // 16
    rows = pl.ds(c * n, n)
    return pltpu.make_async_copy(ao.at[rows], out_h.at[rows, :, 0:D], sem_out.at[1])

  order = []
  for g in range(NG):
    order += [("qk", g)] + ([("pv", g - 1)] if g >= 1 else [])
    order += [("v", g), ("sc", g)] + ([("wo", g - 2)] if g >= 2 else [])
  order += [("pv", NG - 1), ("wo", NG - 2), ("wo", NG - 1)]

  def step(s, mem, first=False):
    hl = jnp.concatenate([mem, ax[s].astype(f32)], axis=0)
    pre = pl.ds(pl.multiple_of(s * PRE, PRE), PRE)
    q, k, v, p, o = {}, {}, {}, {}, {}
    y = [None] * 8
    for op, g in order:
      hs = range(g * G, (g + 1) * G)
      if first and op in ("qk", "v"):
        m = 1 if op == "qk" else 2
        wait(c_w[m][g])
        lax.fori_loop(G // 2 * g, G // 2 * (g + 1), lambda hp, _, m=m: merge(m, hp), None)
      if first and op == "wo":
        wait(c_wo[g])
      for h in hs:
        if op == "qk":
          q[h] = jnp.concatenate([_rnd(_dot(hl[:L - PRE], w1(0, h))), qp[h, pre, :]], axis=0)
          k[h] = _dot(hl, w1(1, h)).astype(bf16)
        elif op == "v":
          v[h] = _dot(hl, w1(2, h)).astype(bf16)
        elif op == "sc":
          sc = jnp.where(mask, _dot_nt(q[h], k[h]) * scale, -1e9)
          e = jnp.exp(sc - jnp.max(sc, axis=-1, keepdims=True))
          p[h] = _rnd(e / jnp.sum(e, axis=-1, keepdims=True))
        elif op == "pv":
          o[h] = _rnd(_dot(p[h], v[h]))
      if op == "wo":
        og = jnp.concatenate([o[h] for h in hs], axis=1)
        for j in range(8):
          t = _dot(og, w2(j, g))
          y[j] = t if y[j] is None else y[j] + t
    yb = jnp.concatenate(y, axis=1).astype(bf16)
    ao[pl.ds(2 * s, 2)] = yb[M:].reshape(2, 16, D)
    return yb[:M].astype(f32)

  with jax.named_scope("a_first"):
    wait(c_a0)
    mem = step(0, mem0[...].astype(f32), first=True)
    wait(c_a1)
  start([c_ob])

  def steps(i, mem):
    s = UNROLL * i + 1
    for u in range(UNROLL):
      mem = step(s + u, mem)
    for u in range(UNROLL):
      @pl.when((s + u) % OUT_CHUNK == OUT_CHUNK - 1)
      def _():
        out_copy((s + u) // OUT_CHUNK).start()
    return mem

  with jax.named_scope("a_loop"):
    lax.fori_loop(0, (NSEG - 1) // UNROLL, steps, mem)

  with jax.named_scope("wait_out"):
    wait(c_ob)
    for c in range(NSEG // OUT_CHUNK):
      out_copy(c).wait()


@functools.partial(jax.jit, static_argnames=("A_seg_len",))
def pallas_concat_heads__memory_aug_recurrent_mem_tr__spectral_gfnet__prompt_kernel(
    A_x, A_mem0, A_Wq, A_Wk, A_Wv, A_Wo, A_seg_len, B_x, B_w_r, B_w_i):
  assert A_seg_len == SEG and A_x.shape == (1, S, D) and A_Wq.shape == (D, H, DH)
  consts = _constants()
  hbm = pl.BlockSpec(memory_space=pltpu.HBM)
  out = pl.pallas_call(
      _kernel,
      out_shape=jax.ShapeDtypeStruct((S // 16, 16, 2 * D), bf16),
      in_specs=[hbm] * 12,
      out_specs=hbm,
      scratch_shapes=[
          pltpu.VMEM((3, 2, H // 2, D // 2, DH), u32),
          pltpu.VMEM((H * DH // 2, D), u32),
          pltpu.VMEM((NSEG, SEG, D), bf16),
          pltpu.VMEM((M, D), bf16),
          pltpu.VMEM((8, 128, D), u32),
          pltpu.VMEM((2, D // 2 + 1, S), bf16),
          pltpu.VMEM((4, 256, 256), bf16),
          pltpu.VMEM((128, 128), bf16),
          pltpu.VMEM((16, 256, 128), bf16),
          pltpu.VMEM((2, KR, S), f32),
          pltpu.VMEM((2, KR, S), f32),
          pltpu.VMEM((S // 16, 16, D), bf16),
          pltpu.VMEM((NSEG, PRE, D), bf16),
          pltpu.VMEM((H, NSEG * PRE, DH), f32),
          pltpu.SemaphoreType.DMA((64,)),
          pltpu.SemaphoreType.DMA((2,)),
      ],
      compiler_params=pltpu.CompilerParams(vmem_limit_bytes=110 * 2**20),
  )(A_x.reshape(NSEG, SEG, D), A_mem0.reshape(M, D),
    A_Wq.reshape(D // 2, 2, H, DH), A_Wk.reshape(D // 2, 2, H, DH), A_Wv.reshape(D // 2, 2, H, DH),
    A_Wo.reshape(H * DH, D), B_x.reshape(S // 16, 16, D),
    B_w_r.T, B_w_i.T, *consts)
  return out.reshape(1, S, 2 * D)
```

```python
import functools

import jax
import jax.numpy as jnp
import numpy as np
from jax import lax
import jax.experimental.pallas as pl
import jax.experimental.pallas.tpu as pltpu

f32, bf16, u32 = jnp.float32, jnp.bfloat16, jnp.uint32

S, D = 2048, 1024
H, DH = 32, 128
M, SEG = 8, 32
L = M + SEG
NSEG = S // SEG
OUT_CHUNK = 8
G = 4
NG = H // G
PRE = 8
UNROLL = 2
KR = D // 2 + 8


def _kd_of_row():
  kd = np.zeros(512, np.int64)
  l = np.arange(64)
  for t in range(4):
    kd[128 * t:128 * t + 64] = t + 8 * l
    kd[128 * t + 64:128 * t + 128] = (8 - t if t else 4) + 8 * l
  return kd


def _spectrum_row_of_residue(r):
  if r < 4:
    return 128 * r
  return 64 if r == 4 else 128 * (8 - r) + 64


def _constants():
  kd = _kd_of_row()
  b = np.arange(128)
  lo = (b < 64)[:, None]
  md = np.zeros((4, 256, 256))
  for t in range(4):
    e = np.exp(-2j * np.pi * np.outer(kd[128 * t:128 * t + 128], b) / D)
    c, s = e.real, e.imag
    if t == 0:
      md[0, :128, :128], md[0, 128:, :128] = np.where(lo, c, 0), np.where(lo, s, 0)
      md[0, :128, 128:], md[0, 128:, 128:] = np.where(lo, 0, c), np.where(lo, 0, s)
      md[0, 128, :128] = (-1.0) ** b
    else:
      sg = np.where(lo, 1.0, -1.0)
      md[t, :128, :128], md[t, 128:, :128] = c, s
      md[t, :128, 128:], md[t, 128:, 128:] = sg * s, -sg * c
  pm = np.zeros((128, 128))
  pm[b, b // 16 + 8 * (b % 16)] = 1.0
  gs = np.zeros((16, 256, 128))
  for a in range(16):
    g = np.exp(-2j * np.pi * np.outer(a + 16 * b, b) / S)
    gs[a, :128], gs[a, 128:] = g.real, g.imag
  cast = lambda a: a.astype(np.float32).astype(jnp.bfloat16)
  return cast(md), cast(pm), cast(gs)


def _dft4(z, sign):
  (ar, ai), (br, bi), (cr, ci), (dr, di) = z
  t0r, t0i, t1r, t1i = ar + cr, ai + ci, ar - cr, ai - ci
  t2r, t2i, t3r, t3i = br + dr, bi + di, br - dr, bi - di
  p = (t1r + t3i, t1i - t3r)
  m = (t1r - t3i, t1i + t3r)
  x1, x3 = (p, m) if sign < 0 else (m, p)
  return [(t0r + t2r, t0i + t2i), x1, (t0r - t2r, t0i - t2i), x3]


def _cmul_w16(z, n, sign):
  zr, zi = z
  if n == 0:
    return z
  if n == 4:
    return (zi, -zr) if sign < 0 else (-zi, zr)
  c = float(np.cos(2 * np.pi * n / 16))
  s = float(sign * np.sin(2 * np.pi * n / 16))
  if n == 2:
    return ((zr + zi) * c, (zi - zr) * c) if sign < 0 else ((zr - zi) * c, (zi + zr) * c)
  if n == 6:
    h = -c
    return ((zi - zr) * h, (zr + zi) * -h) if sign < 0 else ((zr + zi) * -h, (zr - zi) * h)
  return (zr * c - zi * s, zr * s + zi * c)


def _dft16(x, sign):
  t = [_dft4([x[a2], x[4 + a2], x[8 + a2], x[12 + a2]], sign) for a2 in range(4)]
  out = [None] * 16
  for k1 in range(4):
    r = _dft4([_cmul_w16(t[a2][k1], a2 * k1, sign) for a2 in range(4)], sign)
    for k2 in range(4):
      out[k1 + 4 * k2] = r[k2]
  return out


def _rnd(a):
  return a.astype(bf16).astype(f32)


def _dot(a, b):
  return jnp.dot(a, b, preferred_element_type=f32)


def _dot_nt(a, b):
  return lax.dot_general(a, b, (((1,), (1,)), ((), ())), preferred_element_type=f32)


def _kernel(ax_h, mem_h, wq_h, wk_h, wv_h, wo_h, bx_h, wr_h, wi_h, md_h, pm_h, gs_h, out_h,
            wqkv, wo, ax, mem0, bx, wt, md, pm, gs, xs, wf, ao, xq, qp, sem_in, sem_out):
  nsem = [0]

  def group(pairs):
    i = nsem[0]
    nsem[0] += 1
    return [pltpu.make_async_copy(s, d, sem_in.at[i]) for s, d in pairs]

  def wait(copies):
    for c in copies:
      c.wait()

  bx_u = bx_h.bitcast(u32)
  c_const = group([(md_h, md)])
  c_bx = [group([(bx_u.at[:, a, :], bx.at[a]), (gs_h.at[2 * a:2 * a + 2], gs.at[2 * a:2 * a + 2])])
          for a in range(8)]
  c_wt = group([(wr_h, wt.at[0]), (pm_h, pm), (wi_h, wt.at[1])])
  w_u = [w_h.bitcast(u32) for w_h in (wq_h, wk_h, wv_h)]
  wo_u = wo_h.bitcast(u32)

  def w_group(m, g):
    return group([(w_u[m].at[:, par, hp, :], wqkv.at[m, par, hp])
                  for hp in range(G // 2 * g, G // 2 * (g + 1)) for par in range(2)])

  c_w = [[w_group(m, g) for g in range(NG)] for m in range(3)]
  c_wo = [group([(wo_u.at[i * 1024:(i + 1) * 1024, j * 128:(j + 1) * 128],
                  wo.at[j, i * 1024:(i + 1) * 1024]) for j in range(8)]) for i in range(2)]
  c_xq = group([(ax_h.at[:, SEG - PRE:SEG, :], xq)])
  c_a0 = group([(mem_h, mem0), (ax_h.at[0:OUT_CHUNK], ax.at[0:OUT_CHUNK])])
  c_a1 = group([(ax_h.at[OUT_CHUNK:NSEG], ax.at[OUT_CHUNK:NSEG])])

  def start(groups):
    for g in groups:
      for c in g:
        c.start()

  with jax.named_scope("dma_start"):
    start([c_const])
    for a in range(2):
      start([c_bx[a]])

  c_g = [c_w[0][g] + c_w[1][g] + c_w[2][g] for g in range(NG)]

  rc = float(np.sqrt(0.5))

  def col(c):
    return pl.ds(c * 128, 128)

  def dcol(c):
    return pl.ds(pl.multiple_of(c * 128, 128), 128)

  with jax.named_scope("b_fwd"):
    wait(c_const)
    row8 = lax.broadcasted_iota(jnp.int32, (8, 128), 0)

    def fwd(ap, _):
      for a in range(8):
        @pl.when(ap == a)
        def _():
          wait(c_bx[a])
          start([c_bx[a + 2]] if a < 6 else [c_xq] if a == 6 else [c_g[0]])
          if a in (0, 3):
            start([c_wt[:2] if a == 0 else c_wt[2:]])
      for par in range(2):
        a = 2 * ap + par
        w = [bx[ap, :, col(j)] for j in range(8)]
        x = [pltpu.bitcast(v << 16 if par == 0 else v & jnp.uint32(0xFFFF0000), f32) for v in w]
        e0, e1, e2, e3 = x[0] + x[4], x[0] - x[4], x[2] + x[6], x[2] - x[6]
        o0, o1, o2, o3 = x[1] + x[5], x[1] - x[5], x[3] + x[7], x[3] - x[7]
        ep, op = e0 + e2, o0 + o2
        u, v = (o1 - o3) * rc, (o1 + o3) * rc
        z = [(ep + op, ep - op), (e1 + u, v + e3), (e0 - e2, o0 - o2), (e1 - u, v - e3)]
        tt = [_dot_nt(md[t], jnp.concatenate(z[t], axis=1).astype(bf16)) for t in range(4)]
        g = jnp.concatenate([gs[a, :128], gs[a, 128:]], axis=1)
        for t in range(4):
          r = _dot(tt[t].astype(bf16), g)
          rr, ri, ir, ii = r[:128, :128], r[:128, 128:], r[128:, :128], r[128:, 128:]
          if t == 0:
            xs[0, 512:KR, dcol(a)] = jnp.where(row8 == 0, ir[:8], 0.0)
            xs[1, 512:KR, dcol(a)] = jnp.where(row8 == 0, ii[:8], 0.0)
            ir = jnp.concatenate([jnp.where(row8 == 0, 0.0, ir[:8]), ir[8:]], axis=0)
            ii = jnp.concatenate([jnp.where(row8 == 0, 0.0, ii[:8]), ii[8:]], axis=0)
          xs[0, t * 128:(t + 1) * 128, dcol(a)] = rr - ii
          xs[1, t * 128:(t + 1) * 128, dcol(a)] = ri + ir
      return 0

    lax.fori_loop(0, 8, fwd, 0)

  start([c_g[1]])
  with jax.named_scope("b_w"):
    wait(c_wt)

    def wperm(ap, _):
      cols = pl.ds(pl.multiple_of(ap * 512, 512), 512)
      for i in range(2):
        for tile in range(4):
          p = _dot(pm[...], wt[i, tile * 128:(tile + 1) * 128, cols]) * (2.0 / (S * D))
          for r in range(8):
            pr = p[16 * r:16 * r + 16]
            if tile == 0 and r == 0:
              first = lax.broadcasted_iota(jnp.int32, (16, 512), 0) == 0
              pr = jnp.where(first, pr * 0.5, pr)
            r0 = _spectrum_row_of_residue(r) + 16 * tile
            wf[i, r0:r0 + 16, cols] = pr
        ny = wt[i, 512:513, cols].astype(f32) * (1.0 / (S * D))
        wf[i, 512:KR, cols] = jnp.broadcast_to(ny, (8, 512))
      return 0

    lax.fori_loop(0, 4, wperm, 0)

  with jax.named_scope("b_mid"):
    def mid(i, _):
      rows = pl.ds(pl.multiple_of(i * 8, 8), 8)
      y = _dft16([(xs[0, rows, col(a)], xs[1, rows, col(a)]) for a in range(16)], -1)
      z = []
      for c in range(16):
        wr, wi = wf[0, rows, col(c)], wf[1, rows, col(c)]
        yr, yi = y[c]
        z.append((yr * wr - yi * wi, yr * wi + yi * wr))
      q = _dft16(z, 1)
      for a in range(16):
        xs[0, rows, col(a)] = q[a][0]
        xs[1, rows, col(a)] = q[a][1]
      return 0

    lax.fori_loop(0, KR // 8, mid, 0)

  bo_u = out_h.bitcast(u32)
  c_ob = [pltpu.make_async_copy(bx.at[a], bo_u.at[:, a, D:2 * D], sem_out.at[0])
          for a in range(8)]

  with jax.named_scope("b_inv"):
    lane = lax.broadcasted_iota(jnp.int32, (128, 128), 1)

    start([c_g[2]])

    def inv(ap, _):
      for a, g in ((1, 3), (3, 4), (6, 5)):
        @pl.when(ap == a)
        def _():
          start([c_g[g]])
      ys = []
      for par in range(2):
        a = 2 * ap + par
        g = gs[a]
        rs = [_dot_nt(g, jnp.concatenate(
            [xs[0, t * 128:(t + 1) * 128, dcol(a)], xs[1, t * 128:(t + 1) * 128, dcol(a)]],
            axis=0).astype(bf16)) for t in range(4)]
        qn = jnp.concatenate([xs[0, 512:KR, dcol(a)], xs[1, 512:KR, dcol(a)]], axis=1)
        qn = jnp.concatenate([qn, jnp.zeros((120, 256), f32)], axis=0).astype(bf16)
        ny = _dot_nt(jnp.concatenate([g[:128], g[128:]], axis=1), qn)
        z = []
        for t in range(4):
          r = rs[t]
          ur = r[:128, :128] + r[128:, 128:]
          ui = r[:128, 128:] - r[128:, :128]
          if t == 0:
            ui = jnp.where(lane == 0, ny, ui)
          y = _dot(jnp.concatenate([ur, ui], axis=1).astype(bf16), md[t])
          z.append((y[:, :128], y[:, 128:]))
        (z0, z4), (p1, q1), (p2, q2), (p3, q3) = z
        ep, op = z0 + z4, z0 - z4
        e0, e2, o0, o2 = ep + p2, ep - p2, op + q2, op - q2
        e1, e3 = p1 + p3, q1 - q3
        u, v = (p1 - p3) * rc, (q1 + q3) * rc
        o1, o3 = v + u, v - u
        ys.append([e0 + e1, o0 + o1, e2 + e3, o2 + o3, e0 - e1, o0 - o1, e2 - e3, o2 - o3])
      for j in range(8):
        lo = pltpu.bitcast(_rnd(ys[0][j]), u32)
        hi = pltpu.bitcast(_rnd(ys[1][j]), u32)
        bx[ap, :, col(j)] = (lo >> 16) | hi
      return 0

    lax.fori_loop(0, 8, inv, 0)


  def merge(m, hp):
    for r in range(4):
      rows = pl.ds(r * 128, 128)
      a, b = wqkv[m, 0, hp, rows, :], wqkv[m, 1, hp, rows, :]
      wqkv[m, 0, hp, rows, :] = (a & 0xFFFF) | (b << 16)
      wqkv[m, 1, hp, rows, :] = (a >> 16) | (b & jnp.uint32(0xFFFF0000))

  def w1(m, h):
    return pltpu.bitcast(wqkv[m, h % 2, h // 2], bf16)

  def w2(j, g):
    return pltpu.bitcast(wo[j, g * G * 64:(g + 1) * G * 64], bf16)

  with jax.named_scope("q_pre"):
    wait(c_xq)
    for g in range(NG):
      wait(c_g[g])
      start({0: [c_g[6]], 2: [c_g[7]], 4: [c_a0, c_wo[0]], 6: [c_wo[1]]}.get(g, []))

      def q_pre(hp, _):
        for m in range(3):
          merge(m, hp)
        xv = xq[...].reshape(NSEG * PRE, D)
        for par in range(2):
          qp[2 * hp + par] = _rnd(_dot(xv, pltpu.bitcast(wqkv[0, par, hp], bf16)))
        return 0

      lax.fori_loop(G // 2 * g, G // 2 * (g + 1), q_pre, 0)

  row = lax.broadcasted_iota(jnp.int32, (L, L), 0)
  colm = lax.broadcasted_iota(jnp.int32, (L, L), 1)
  mask = (row < M) | (row >= colm)
  scale = DH ** -0.5

  def out_copy(c):
    n = OUT_CHUNK * SEG // 16
    rows = pl.ds(c * n, n)
    return pltpu.make_async_copy(ao.at[rows], out_h.at[rows, :, 0:D], sem_out.at[1])

  order = []
  for g in range(NG):
    order += [("qk", g)] + ([("pv", g - 1)] if g >= 1 else [])
    order += [("v", g), ("sc", g)] + ([("wo", g - 2)] if g >= 2 else [])
  order += [("pv", NG - 1), ("wo", NG - 2), ("wo", NG - 1)]

  def step(s, mem):
    hl = jnp.concatenate([mem, ax[s].astype(f32)], axis=0)
    pre = pl.ds(pl.multiple_of(s * PRE, PRE), PRE)
    q, k, v, p, o = {}, {}, {}, {}, {}
    y = [None] * 8
    for op, g in order:
      hs = range(g * G, (g + 1) * G)
      for h in hs:
        if op == "qk":
          q[h] = jnp.concatenate([_rnd(_dot(hl[:L - PRE], w1(0, h))), qp[h, pre, :]], axis=0)
          k[h] = _dot(hl, w1(1, h)).astype(bf16)
        elif op == "v":
          v[h] = _dot(hl, w1(2, h)).astype(bf16)
        elif op == "sc":
          sc = jnp.where(mask, _dot_nt(q[h], k[h]) * scale, -1e9)
          e = jnp.exp(sc - jnp.max(sc, axis=-1, keepdims=True))
          p[h] = _rnd(e / jnp.sum(e, axis=-1, keepdims=True))
        elif op == "pv":
          o[h] = _rnd(_dot(p[h], v[h]))
      if op == "wo":
        og = jnp.concatenate([o[h] for h in hs], axis=1)
        for j in range(8):
          t = _dot(og, w2(j, g))
          y[j] = t if y[j] is None else y[j] + t
    yb = jnp.concatenate(y, axis=1).astype(bf16)
    ao[pl.ds(2 * s, 2)] = yb[M:].reshape(2, 16, D)
    return yb[:M].astype(f32)

  with jax.named_scope("a_wait"):
    wait(c_a0 + c_wo[0] + c_wo[1])
  start([c_a1, c_ob])

  def steps(i, mem):
    s = UNROLL * i

    @pl.when(s == OUT_CHUNK)
    def _():
      wait(c_a1)

    for u in range(UNROLL):
      mem = step(s + u, mem)

    @pl.when((s + UNROLL) % OUT_CHUNK == 0)
    def _():
      out_copy(s // OUT_CHUNK).start()

    return mem

  with jax.named_scope("a_loop"):
    lax.fori_loop(0, NSEG // UNROLL, steps, mem0[...].astype(f32))

  with jax.named_scope("wait_out"):
    wait(c_ob)
    for c in range(NSEG // OUT_CHUNK):
      out_copy(c).wait()


@functools.partial(jax.jit, static_argnames=("A_seg_len",))
def pallas_concat_heads__memory_aug_recurrent_mem_tr__spectral_gfnet__prompt_kernel(
    A_x, A_mem0, A_Wq, A_Wk, A_Wv, A_Wo, A_seg_len, B_x, B_w_r, B_w_i):
  assert A_seg_len == SEG and A_x.shape == (1, S, D) and A_Wq.shape == (D, H, DH)
  consts = _constants()
  hbm = pl.BlockSpec(memory_space=pltpu.HBM)
  out = pl.pallas_call(
      _kernel,
      out_shape=jax.ShapeDtypeStruct((S // 16, 16, 2 * D), bf16),
      in_specs=[hbm] * 12,
      out_specs=hbm,
      scratch_shapes=[
          pltpu.VMEM((3, 2, H // 2, D // 2, DH), u32),
          pltpu.VMEM((D // 128, H * DH // 2, 128), u32),
          pltpu.VMEM((NSEG, SEG, D), bf16),
          pltpu.VMEM((M, D), bf16),
          pltpu.VMEM((8, 128, D), u32),
          pltpu.VMEM((2, D // 2 + 1, S), bf16),
          pltpu.VMEM((4, 256, 256), bf16),
          pltpu.VMEM((128, 128), bf16),
          pltpu.VMEM((16, 256, 128), bf16),
          pltpu.VMEM((2, KR, S), f32),
          pltpu.VMEM((2, KR, S), f32),
          pltpu.VMEM((S // 16, 16, D), bf16),
          pltpu.VMEM((NSEG, PRE, D), bf16),
          pltpu.VMEM((H, NSEG * PRE, DH), f32),
          pltpu.SemaphoreType.DMA((64,)),
          pltpu.SemaphoreType.DMA((2,)),
      ],
      compiler_params=pltpu.CompilerParams(vmem_limit_bytes=110 * 2**20),
  )(A_x.reshape(NSEG, SEG, D), A_mem0.reshape(M, D),
    A_Wq.reshape(D // 2, 2, H, DH), A_Wk.reshape(D // 2, 2, H, DH), A_Wv.reshape(D // 2, 2, H, DH),
    A_Wo.reshape(H * DH, D), B_x.reshape(S // 16, 16, D),
    B_w_r.T, B_w_i.T, *consts)
  return out.reshape(1, S, 2 * D)
```

```python
import functools

import jax
import jax.numpy as jnp
import numpy as np
from jax import lax
import jax.experimental.pallas as pl
import jax.experimental.pallas.tpu as pltpu

f32, bf16, u32 = jnp.float32, jnp.bfloat16, jnp.uint32

S, D = 2048, 1024
H, DH = 32, 128
M, SEG = 8, 32
L = M + SEG
NSEG = S // SEG
OUT_CHUNK = 8
G = 4
NG = H // G
PRE = 8
KPRE = 8
UNROLL = 2
KR = D // 2 + 8


def _kd_of_row():
  kd = np.zeros(512, np.int64)
  l = np.arange(64)
  for t in range(4):
    kd[128 * t:128 * t + 64] = t + 8 * l
    kd[128 * t + 64:128 * t + 128] = (8 - t if t else 4) + 8 * l
  return kd


def _spectrum_row_of_residue(r):
  if r < 4:
    return 128 * r
  return 64 if r == 4 else 128 * (8 - r) + 64


def _constants():
  kd = _kd_of_row()
  b = np.arange(128)
  lo = (b < 64)[:, None]
  md = np.zeros((4, 256, 256))
  for t in range(4):
    e = np.exp(-2j * np.pi * np.outer(kd[128 * t:128 * t + 128], b) / D)
    c, s = e.real, e.imag
    if t == 0:
      md[0, :128, :128], md[0, 128:, :128] = np.where(lo, c, 0), np.where(lo, s, 0)
      md[0, :128, 128:], md[0, 128:, 128:] = np.where(lo, 0, c), np.where(lo, 0, s)
      md[0, 128, :128] = (-1.0) ** b
    else:
      sg = np.where(lo, 1.0, -1.0)
      md[t, :128, :128], md[t, 128:, :128] = c, s
      md[t, :128, 128:], md[t, 128:, 128:] = sg * s, -sg * c
  pm = np.zeros((128, 128))
  pm[b, b // 16 + 8 * (b % 16)] = 1.0
  gs = np.zeros((16, 256, 128))
  for a in range(16):
    g = np.exp(-2j * np.pi * np.outer(a + 16 * b, b) / S)
    gs[a, :128], gs[a, 128:] = g.real, g.imag
  cast = lambda a: a.astype(np.float32).astype(jnp.bfloat16)
  return cast(md), cast(pm), cast(gs)


def _dft4(z, sign):
  (ar, ai), (br, bi), (cr, ci), (dr, di) = z
  t0r, t0i, t1r, t1i = ar + cr, ai + ci, ar - cr, ai - ci
  t2r, t2i, t3r, t3i = br + dr, bi + di, br - dr, bi - di
  p = (t1r + t3i, t1i - t3r)
  m = (t1r - t3i, t1i + t3r)
  x1, x3 = (p, m) if sign < 0 else (m, p)
  return [(t0r + t2r, t0i + t2i), x1, (t0r - t2r, t0i - t2i), x3]


def _cmul_w16(z, n, sign):
  zr, zi = z
  if n == 0:
    return z
  if n == 4:
    return (zi, -zr) if sign < 0 else (-zi, zr)
  c = float(np.cos(2 * np.pi * n / 16))
  s = float(sign * np.sin(2 * np.pi * n / 16))
  if n == 2:
    return ((zr + zi) * c, (zi - zr) * c) if sign < 0 else ((zr - zi) * c, (zi + zr) * c)
  if n == 6:
    h = -c
    return ((zi - zr) * h, (zr + zi) * -h) if sign < 0 else ((zr + zi) * -h, (zr - zi) * h)
  return (zr * c - zi * s, zr * s + zi * c)


def _dft16(x, sign):
  t = [_dft4([x[a2], x[4 + a2], x[8 + a2], x[12 + a2]], sign) for a2 in range(4)]
  out = [None] * 16
  for k1 in range(4):
    r = _dft4([_cmul_w16(t[a2][k1], a2 * k1, sign) for a2 in range(4)], sign)
    for k2 in range(4):
      out[k1 + 4 * k2] = r[k2]
  return out


def _rnd(a):
  return a.astype(bf16).astype(f32)


def _dot(a, b):
  return jnp.dot(a, b, preferred_element_type=f32)


def _dot_nt(a, b):
  return lax.dot_general(a, b, (((1,), (1,)), ((), ())), preferred_element_type=f32)


def _kernel(ax_h, mem_h, wq_h, wk_h, wv_h, wo_h, bx_h, wr_h, wi_h, md_h, pm_h, gs_h, out_h,
            wqkv, wo, ax, mem0, bx, wt, md, pm, gs, xs, wf, ao, xq, qp, kp, sem_in, sem_out):
  nsem = [0]

  def group(pairs):
    i = nsem[0]
    nsem[0] += 1
    return [pltpu.make_async_copy(s, d, sem_in.at[i]) for s, d in pairs]

  def wait(copies):
    for c in copies:
      c.wait()

  bx_u = bx_h.bitcast(u32)
  c_const = group([(md_h, md)])
  c_bx = [group([(bx_u.at[:, a, :], bx.at[a]), (gs_h.at[2 * a:2 * a + 2], gs.at[2 * a:2 * a + 2])])
          for a in range(8)]
  c_wt = group([(wr_h, wt.at[0]), (pm_h, pm), (wi_h, wt.at[1])])
  w_u = [w_h.bitcast(u32) for w_h in (wq_h, wk_h, wv_h)]
  wo_u = wo_h.bitcast(u32)

  def w_group(m, g):
    return group([(w_u[m].at[:, par, hp, :], wqkv.at[m, par, hp])
                  for hp in range(4 * g, 4 * g + 4) for par in range(2)])

  c_w = [w_group(m, g) for m in range(3) for g in range(4)]
  c_wo = [group([(wo_u.at[i * 1024:(i + 1) * 1024, j * 128:(j + 1) * 128],
                  wo.at[j, i * 1024:(i + 1) * 1024]) for j in range(8)]) for i in range(2)]
  c_xq = group([(ax_h.at[:, SEG - PRE:SEG, :], xq)])
  c_a0 = group([(mem_h, mem0), (ax_h.at[0:OUT_CHUNK], ax.at[0:OUT_CHUNK])])
  c_a1 = group([(ax_h.at[OUT_CHUNK:NSEG], ax.at[OUT_CHUNK:NSEG])])

  def start(groups):
    for g in groups:
      for c in g:
        c.start()

  with jax.named_scope("dma_start"):
    start([c_const])
    for a in range(2):
      start([c_bx[a]])


  def at_step(i, table):
    for n, fn in table.items():
      pl.when(i == n)(fn)

  def merge(m, hp):
    for r in range(4):
      rows = pl.ds(r * 128, 128)
      a, b = wqkv[m, 0, hp, rows, :], wqkv[m, 1, hp, rows, :]
      wqkv[m, 0, hp, rows, :] = (a & 0xFFFF) | (b << 16)
      wqkv[m, 1, hp, rows, :] = (a >> 16) | (b & jnp.uint32(0xFFFF0000))

  def project(m, hp, dst):
    xv = xq[...].reshape(NSEG * PRE, D)
    for par in range(2):
      dst[2 * hp + par] = _rnd(_dot(xv, pltpu.bitcast(wqkv[m, par, hp], bf16)))

  rc = float(np.sqrt(0.5))

  def col(c):
    return pl.ds(c * 128, 128)

  def dcol(c):
    return pl.ds(pl.multiple_of(c * 128, 128), 128)

  with jax.named_scope("b_fwd"):
    wait(c_const)
    row8 = lax.broadcasted_iota(jnp.int32, (8, 128), 0)

    def fwd(it, _):
      def fetch(n):
        wait(c_bx[2 * n] + c_bx[2 * n + 1])
        start([[c_bx[2], c_bx[3], c_wt[:2]], [c_bx[4], c_bx[5]], [c_bx[6], c_bx[7], c_wt[2:]],
               [c_xq, c_w[0]]][n])

      at_step(it, {n: functools.partial(fetch, n) for n in range(4)})
      for u in range(4):
        a, ap, par = 4 * it + u, 2 * it + u // 2, u % 2
        w = [bx[ap, :, col(j)] for j in range(8)]
        x = [pltpu.bitcast(v << 16 if par == 0 else v & jnp.uint32(0xFFFF0000), f32) for v in w]
        e0, e1, e2, e3 = x[0] + x[4], x[0] - x[4], x[2] + x[6], x[2] - x[6]
        o0, o1, o2, o3 = x[1] + x[5], x[1] - x[5], x[3] + x[7], x[3] - x[7]
        ep, op = e0 + e2, o0 + o2
        u, v = (o1 - o3) * rc, (o1 + o3) * rc
        z = [(ep + op, ep - op), (e1 + u, v + e3), (e0 - e2, o0 - o2), (e1 - u, v - e3)]
        tt = [_dot_nt(md[t], jnp.concatenate(z[t], axis=1).astype(bf16)) for t in range(4)]
        g = jnp.concatenate([gs[a, :128], gs[a, 128:]], axis=1)
        for t in range(4):
          r = _dot(tt[t].astype(bf16), g)
          rr, ri, ir, ii = r[:128, :128], r[:128, 128:], r[128:, :128], r[128:, 128:]
          if t == 0:
            xs[0, 512:KR, dcol(a)] = jnp.where(row8 == 0, ir[:8], 0.0)
            xs[1, 512:KR, dcol(a)] = jnp.where(row8 == 0, ii[:8], 0.0)
            ir = jnp.concatenate([jnp.where(row8 == 0, 0.0, ir[:8]), ir[8:]], axis=0)
            ii = jnp.concatenate([jnp.where(row8 == 0, 0.0, ii[:8]), ii[8:]], axis=0)
          xs[0, t * 128:(t + 1) * 128, dcol(a)] = rr - ii
          xs[1, t * 128:(t + 1) * 128, dcol(a)] = ri + ir
      return 0

    lax.fori_loop(0, 4, fwd, 0)

  start([c_w[1]])
  with jax.named_scope("b_w"):
    wait(c_wt)

    def wperm(ap, _):
      cols = pl.ds(pl.multiple_of(ap * 1024, 1024), 1024)
      for i in range(2):
        for tile in range(4):
          p = _dot(pm[...], wt[i, tile * 128:(tile + 1) * 128, cols]) * (2.0 / (S * D))
          for r in range(8):
            pr = p[16 * r:16 * r + 16]
            if tile == 0 and r == 0:
              first = lax.broadcasted_iota(jnp.int32, (16, 1024), 0) == 0
              pr = jnp.where(first, pr * 0.5, pr)
            r0 = _spectrum_row_of_residue(r) + 16 * tile
            wf[i, r0:r0 + 16, cols] = pr
        ny = wt[i, 512:513, cols].astype(f32) * (1.0 / (S * D))
        wf[i, 512:KR, cols] = jnp.broadcast_to(ny, (8, 1024))
      return 0

    lax.fori_loop(0, 2, wperm, 0, unroll=False)

  with jax.named_scope("b_mid"):
    def mid(i):
      rows = pl.ds(pl.multiple_of(i * 8, 8), 8)
      y = _dft16([(xs[0, rows, col(a)], xs[1, rows, col(a)]) for a in range(16)], -1)
      z = []
      for c in range(16):
        wr, wi = wf[0, rows, col(c)], wf[1, rows, col(c)]
        yr, yi = y[c]
        z.append((yr * wr - yi * wi, yr * wi + yi * wr))
      q = _dft16(z, 1)
      for a in range(16):
        xs[0, rows, col(a)] = q[a][0]
        xs[1, rows, col(a)] = q[a][1]

    def mid_and_q(hp, _):
      merge(0, hp)
      for u in range(16):
        par, n = u // 8, u % 8
        xv = xq[8 * n:8 * n + 8].reshape(8 * PRE, D)
        qp[2 * hp + par, 8 * n * PRE:(8 * n + 8) * PRE] = _rnd(
            _dot(xv, pltpu.bitcast(wqkv[0, par, hp], bf16)))
        mid(16 * hp + u)
      return 0

    start([c_w[2], c_w[3]])
    mid(KR // 8 - 1)
    wait(c_xq + c_w[0])
    lax.fori_loop(0, 4, mid_and_q, 0)

  bo_u = out_h.bitcast(u32)
  c_ob = [pltpu.make_async_copy(bx.at[a], bo_u.at[:, a, D:2 * D], sem_out.at[0])
          for a in range(8)]

  with jax.named_scope("b_inv"):
    lane = lax.broadcasted_iota(jnp.int32, (128, 128), 1)

    def inv(ap):
      ys = []
      for par in range(2):
        a = 2 * ap + par
        g = gs[a]
        rs = [_dot_nt(g, jnp.concatenate(
            [xs[0, t * 128:(t + 1) * 128, dcol(a)], xs[1, t * 128:(t + 1) * 128, dcol(a)]],
            axis=0).astype(bf16)) for t in range(4)]
        qn = jnp.concatenate([xs[0, 512:KR, dcol(a)], xs[1, 512:KR, dcol(a)]], axis=1)
        qn = jnp.concatenate([qn, jnp.zeros((120, 256), f32)], axis=0).astype(bf16)
        ny = _dot_nt(jnp.concatenate([g[:128], g[128:]], axis=1), qn)
        z = []
        for t in range(4):
          r = rs[t]
          ur = r[:128, :128] + r[128:, 128:]
          ui = r[:128, 128:] - r[128:, :128]
          if t == 0:
            ui = jnp.where(lane == 0, ny, ui)
          y = _dot(jnp.concatenate([ur, ui], axis=1).astype(bf16), md[t])
          z.append((y[:, :128], y[:, 128:]))
        (z0, z4), (p1, q1), (p2, q2), (p3, q3) = z
        ep, op = z0 + z4, z0 - z4
        e0, e2, o0, o2 = ep + p2, ep - p2, op + q2, op - q2
        e1, e3 = p1 + p3, q1 - q3
        u, v = (p1 - p3) * rc, (q1 + q3) * rc
        o1, o3 = v + u, v - u
        ys.append([e0 + e1, o0 + o1, e2 + e3, o2 + o3, e0 - e1, o0 - o1, e2 - e3, o2 - o3])
      for j in range(8):
        lo = pltpu.bitcast(_rnd(ys[0][j]), u32)
        hi = pltpu.bitcast(_rnd(ys[1][j]), u32)
        bx[ap, :, col(j)] = (lo >> 16) | hi

    def inv2(it, _):
      at_step(it, {n: functools.partial(start, [c_w[4 + n]]) for n in range(4)})
      inv(2 * it)
      inv(2 * it + 1)
      return 0

    lax.fori_loop(0, 4, inv2, 0)


  def w1(m, h):
    return pltpu.bitcast(wqkv[m, h % 2, h // 2], bf16)

  def w2(j, g):
    return pltpu.bitcast(wo[j, g * G * 64:(g + 1) * G * 64], bf16)

  with jax.named_scope("q_pre"):
    def q_pre(it, _):
      def fetch(n):
        wait(c_w[4 + n] + (c_w[1] + c_w[2] + c_w[3] if n == 0 else []))
        start([[c_w[8], c_w[9]], [c_w[10], c_w[11]], [c_a0, c_wo[0]], [c_wo[1]]][n])

      at_step(it, {n: functools.partial(fetch, n) for n in range(4)})
      for u in range(3):
        merge(0, 4 + 3 * it + u)
        project(0, 4 + 3 * it + u, qp)
      for u in range(4):
        merge(1, 4 * it + u)
      return 0

    lax.fori_loop(0, 4, q_pre, 0)

  with jax.named_scope("k_pre"):
    wait(c_w[8] + c_w[9] + c_w[10] + c_w[11])

    def k_pre(it, _):
      for u in range(KPRE // 4):
        project(1, KPRE // 4 * it + u, kp)
      for u in range(8):
        merge(2, 8 * it + u)
      return 0

    lax.fori_loop(0, 2, k_pre, 0)

  row = lax.broadcasted_iota(jnp.int32, (L, L), 0)
  colm = lax.broadcasted_iota(jnp.int32, (L, L), 1)
  mask = (row < M) | (row >= colm)
  scale = DH ** -0.5

  def out_copy(c):
    n = OUT_CHUNK * SEG // 16
    rows = pl.ds(c * n, n)
    return pltpu.make_async_copy(ao.at[rows], out_h.at[rows, :, 0:D], sem_out.at[1])

  order = []
  for g in range(NG):
    order += [("qk", g)] + ([("pv", g - 1)] if g >= 1 else [])
    order += [("v", g), ("sc", g)] + ([("wo", g - 2)] if g >= 2 else [])
  order += [("pv", NG - 1), ("wo", NG - 2), ("wo", NG - 1)]

  def step(s, mem):
    hl = jnp.concatenate([mem, ax[s].astype(f32)], axis=0)
    pre = pl.ds(pl.multiple_of(s * PRE, PRE), PRE)
    q, k, v, p, o = {}, {}, {}, {}, {}
    y = [None] * 8
    for op, g in order:
      hs = range(g * G, (g + 1) * G)
      for h in hs:
        if op == "qk":
          q[h] = jnp.concatenate([_rnd(_dot(hl[:L - PRE], w1(0, h))), qp[h, pre, :]], axis=0)
          if h < KPRE:
            k[h] = jnp.concatenate([_dot(hl[:L - PRE], w1(1, h)), kp[h, pre, :]], axis=0).astype(bf16)
          else:
            k[h] = _dot(hl, w1(1, h)).astype(bf16)
        elif op == "v":
          v[h] = _dot(hl, w1(2, h)).astype(bf16)
        elif op == "sc":
          sc = jnp.where(mask, _dot_nt(q[h], k[h]) * scale, -1e9)
          e = jnp.exp(sc - jnp.max(sc, axis=-1, keepdims=True))
          p[h] = _rnd(e / jnp.sum(e, axis=-1, keepdims=True))
        elif op == "pv":
          o[h] = _rnd(_dot(p[h], v[h]))
      if op == "wo":
        og = jnp.concatenate([o[h] for h in hs], axis=1)
        for j in range(8):
          t = _dot(og, w2(j, g))
          y[j] = t if y[j] is None else y[j] + t
    yb = jnp.concatenate(y, axis=1).astype(bf16)
    ao[pl.ds(2 * s, 2)] = yb[M:].reshape(2, 16, D)
    return yb[:M].astype(f32)

  with jax.named_scope("a_wait"):
    wait(c_a0 + c_wo[0] + c_wo[1])
  start([c_a1, c_ob])

  def steps(i, mem):
    s = UNROLL * i

    @pl.when(s == OUT_CHUNK)
    def _():
      wait(c_a1)

    for u in range(UNROLL):
      mem = step(s + u, mem)

    @pl.when((s + UNROLL) % OUT_CHUNK == 0)
    def _():
      out_copy(s // OUT_CHUNK).start()

    return mem

  with jax.named_scope("a_loop"):
    lax.fori_loop(0, NSEG // UNROLL, steps, mem0[...].astype(f32))

  with jax.named_scope("wait_out"):
    wait(c_ob)
    for c in range(NSEG // OUT_CHUNK):
      out_copy(c).wait()


@functools.partial(jax.jit, static_argnames=("A_seg_len",))
def pallas_concat_heads__memory_aug_recurrent_mem_tr__spectral_gfnet__prompt_kernel(
    A_x, A_mem0, A_Wq, A_Wk, A_Wv, A_Wo, A_seg_len, B_x, B_w_r, B_w_i):
  assert A_seg_len == SEG and A_x.shape == (1, S, D) and A_Wq.shape == (D, H, DH)
  consts = _constants()
  hbm = pl.BlockSpec(memory_space=pltpu.HBM)
  out = pl.pallas_call(
      _kernel,
      out_shape=jax.ShapeDtypeStruct((S // 16, 16, 2 * D), bf16),
      in_specs=[hbm] * 12,
      out_specs=hbm,
      scratch_shapes=[
          pltpu.VMEM((3, 2, H // 2, D // 2, DH), u32),
          pltpu.VMEM((D // 128, H * DH // 2, 128), u32),
          pltpu.VMEM((NSEG, SEG, D), bf16),
          pltpu.VMEM((M, D), bf16),
          pltpu.VMEM((8, 128, D), u32),
          pltpu.VMEM((2, D // 2 + 1, S), bf16),
          pltpu.VMEM((4, 256, 256), bf16),
          pltpu.VMEM((128, 128), bf16),
          pltpu.VMEM((16, 256, 128), bf16),
          pltpu.VMEM((2, KR, S), f32),
          pltpu.VMEM((2, KR, S), f32),
          pltpu.VMEM((S // 16, 16, D), bf16),
          pltpu.VMEM((NSEG, PRE, D), bf16),
          pltpu.VMEM((H, NSEG * PRE, DH), f32),
          pltpu.VMEM((KPRE, NSEG * PRE, DH), f32),
          pltpu.SemaphoreType.DMA((64,)),
          pltpu.SemaphoreType.DMA((2,)),
      ],
      compiler_params=pltpu.CompilerParams(vmem_limit_bytes=110 * 2**20),
  )(A_x.reshape(NSEG, SEG, D), A_mem0.reshape(M, D),
    A_Wq.reshape(D // 2, 2, H, DH), A_Wk.reshape(D // 2, 2, H, DH), A_Wv.reshape(D // 2, 2, H, DH),
    A_Wo.reshape(H * DH, D), B_x.reshape(S // 16, 16, D),
    B_w_r.T, B_w_i.T, *consts)
  return out.reshape(1, S, 2 * D)
```

```python
import functools

import jax
import jax.numpy as jnp
import numpy as np
from jax import lax
import jax.experimental.pallas as pl
import jax.experimental.pallas.tpu as pltpu

f32, bf16, u32 = jnp.float32, jnp.bfloat16, jnp.uint32

S, D = 2048, 1024
H, DH = 32, 128
M, SEG = 8, 32
L = M + SEG
NSEG = S // SEG
OUT_CHUNK = 8
G = 4
NG = H // G
PRE = 8
KPRE = 8
UNROLL = 2
KR = D // 2 + 8


def _kd_of_row():
  kd = np.zeros(512, np.int64)
  l = np.arange(64)
  for t in range(4):
    kd[128 * t:128 * t + 64] = t + 8 * l
    kd[128 * t + 64:128 * t + 128] = (8 - t if t else 4) + 8 * l
  return kd


def _spectrum_row_of_residue(r):
  if r < 4:
    return 128 * r
  return 64 if r == 4 else 128 * (8 - r) + 64


def _constants():
  kd = _kd_of_row()
  b = np.arange(128)
  lo = (b < 64)[:, None]
  md = np.zeros((4, 256, 256))
  for t in range(4):
    e = np.exp(-2j * np.pi * np.outer(kd[128 * t:128 * t + 128], b) / D)
    c, s = e.real, e.imag
    if t == 0:
      md[0, :128, :128], md[0, 128:, :128] = np.where(lo, c, 0), np.where(lo, s, 0)
      md[0, :128, 128:], md[0, 128:, 128:] = np.where(lo, 0, c), np.where(lo, 0, s)
      md[0, 128, :128] = (-1.0) ** b
    else:
      sg = np.where(lo, 1.0, -1.0)
      md[t, :128, :128], md[t, 128:, :128] = c, s
      md[t, :128, 128:], md[t, 128:, 128:] = sg * s, -sg * c
  pm = np.zeros((128, 128))
  pm[b, b // 16 + 8 * (b % 16)] = 1.0
  gs = np.zeros((16, 256, 128))
  for a in range(16):
    g = np.exp(-2j * np.pi * np.outer(a + 16 * b, b) / S)
    gs[a, :128], gs[a, 128:] = g.real, g.imag
  cast = lambda a: a.astype(np.float32).astype(jnp.bfloat16)
  return cast(md), cast(pm), cast(gs)


def _dft4(z, sign):
  (ar, ai), (br, bi), (cr, ci), (dr, di) = z
  t0r, t0i, t1r, t1i = ar + cr, ai + ci, ar - cr, ai - ci
  t2r, t2i, t3r, t3i = br + dr, bi + di, br - dr, bi - di
  p = (t1r + t3i, t1i - t3r)
  m = (t1r - t3i, t1i + t3r)
  x1, x3 = (p, m) if sign < 0 else (m, p)
  return [(t0r + t2r, t0i + t2i), x1, (t0r - t2r, t0i - t2i), x3]


def _cmul_w16(z, n, sign):
  zr, zi = z
  if n == 0:
    return z
  if n == 4:
    return (zi, -zr) if sign < 0 else (-zi, zr)
  c = float(np.cos(2 * np.pi * n / 16))
  s = float(sign * np.sin(2 * np.pi * n / 16))
  if n == 2:
    return ((zr + zi) * c, (zi - zr) * c) if sign < 0 else ((zr - zi) * c, (zi + zr) * c)
  if n == 6:
    h = -c
    return ((zi - zr) * h, (zr + zi) * -h) if sign < 0 else ((zr + zi) * -h, (zr - zi) * h)
  return (zr * c - zi * s, zr * s + zi * c)


def _dft16(x, sign):
  t = [_dft4([x[a2], x[4 + a2], x[8 + a2], x[12 + a2]], sign) for a2 in range(4)]
  out = [None] * 16
  for k1 in range(4):
    r = _dft4([_cmul_w16(t[a2][k1], a2 * k1, sign) for a2 in range(4)], sign)
    for k2 in range(4):
      out[k1 + 4 * k2] = r[k2]
  return out


def _rnd(a):
  return a.astype(bf16).astype(f32)


def _dot(a, b):
  return jnp.dot(a, b, preferred_element_type=f32)


def _dot_nt(a, b):
  return lax.dot_general(a, b, (((1,), (1,)), ((), ())), preferred_element_type=f32)


def _kernel(ax_h, mem_h, wq_h, wk_h, wv_h, wo_h, bx_h, wr_h, wi_h, md_h, pm_h, gs_h, out_h,
            wqkv, wo, ax, mem0, bx, wt, md, pm, gs, xs, wf, ao, xq, qp, kp, sem_in, sem_out):
  nsem = [0]

  def group(pairs):
    i = nsem[0]
    nsem[0] += 1
    return [pltpu.make_async_copy(s, d, sem_in.at[i]) for s, d in pairs]

  def wait(copies):
    for c in copies:
      c.wait()

  bx_u = bx_h.bitcast(u32)
  c_const = group([(md_h, md)])
  c_bx = [group([(bx_u.at[:, a, :], bx.at[a]), (gs_h.at[2 * a:2 * a + 2], gs.at[2 * a:2 * a + 2])])
          for a in range(8)]
  c_wt = group([(wr_h, wt.at[0]), (pm_h, pm), (wi_h, wt.at[1])])
  w_u = [w_h.bitcast(u32) for w_h in (wq_h, wk_h, wv_h)]
  wo_u = wo_h.bitcast(u32)

  def w_group(m, g):
    return group([(w_u[m].at[:, par, hp, :], wqkv.at[m, par, hp])
                  for hp in range(4 * g, 4 * g + 4) for par in range(2)])

  c_w = [w_group(m, g) for m in range(3) for g in range(4)]
  c_wo = [group([(wo_u.at[i * 1024:(i + 1) * 1024, j * 128:(j + 1) * 128],
                  wo.at[j, i * 1024:(i + 1) * 1024]) for j in range(8)]) for i in range(2)]
  c_xq = group([(ax_h.at[:, SEG - PRE:SEG, :], xq)])
  c_a0 = group([(mem_h, mem0), (ax_h.at[0:OUT_CHUNK], ax.at[0:OUT_CHUNK])])
  c_a1 = group([(ax_h.at[OUT_CHUNK:NSEG], ax.at[OUT_CHUNK:NSEG])])

  def start(groups):
    for g in groups:
      for c in g:
        c.start()

  with jax.named_scope("dma_start"):
    start([c_const])
    start(c_bx + [c_wt, c_xq] + c_w[0:4])

  def at_step(i, table):
    for n, fn in table.items():
      pl.when(i == n)(fn)

  def merge(m, hp):
    for r in range(4):
      rows = pl.ds(r * 128, 128)
      a, b = wqkv[m, 0, hp, rows, :], wqkv[m, 1, hp, rows, :]
      wqkv[m, 0, hp, rows, :] = (a & 0xFFFF) | (b << 16)
      wqkv[m, 1, hp, rows, :] = (a >> 16) | (b & jnp.uint32(0xFFFF0000))

  def project(m, hp, dst):
    xv = xq[...].reshape(NSEG * PRE, D)
    for par in range(2):
      dst[2 * hp + par] = _rnd(_dot(xv, pltpu.bitcast(wqkv[m, par, hp], bf16)))

  rc = float(np.sqrt(0.5))

  def col(c):
    return pl.ds(c * 128, 128)

  def dcol(c):
    return pl.ds(pl.multiple_of(c * 128, 128), 128)

  with jax.named_scope("b_fwd"):
    wait(c_const)
    row8 = lax.broadcasted_iota(jnp.int32, (8, 128), 0)

    def fwd(it, _):
      at_step(it, {n: functools.partial(wait, c_bx[2 * n] + c_bx[2 * n + 1]) for n in range(4)})
      for u in range(4):
        a, ap, par = 4 * it + u, 2 * it + u // 2, u % 2
        w = [bx[ap, :, col(j)] for j in range(8)]
        x = [pltpu.bitcast(v << 16 if par == 0 else v & jnp.uint32(0xFFFF0000), f32) for v in w]
        e0, e1, e2, e3 = x[0] + x[4], x[0] - x[4], x[2] + x[6], x[2] - x[6]
        o0, o1, o2, o3 = x[1] + x[5], x[1] - x[5], x[3] + x[7], x[3] - x[7]
        ep, op = e0 + e2, o0 + o2
        u, v = (o1 - o3) * rc, (o1 + o3) * rc
        z = [(ep + op, ep - op), (e1 + u, v + e3), (e0 - e2, o0 - o2), (e1 - u, v - e3)]
        tt = [_dot_nt(md[t], jnp.concatenate(z[t], axis=1).astype(bf16)) for t in range(4)]
        g = jnp.concatenate([gs[a, :128], gs[a, 128:]], axis=1)
        for t in range(4):
          r = _dot(tt[t].astype(bf16), g)
          rr, ri, ir, ii = r[:128, :128], r[:128, 128:], r[128:, :128], r[128:, 128:]
          if t == 0:
            xs[0, 512:KR, dcol(a)] = jnp.where(row8 == 0, ir[:8], 0.0)
            xs[1, 512:KR, dcol(a)] = jnp.where(row8 == 0, ii[:8], 0.0)
            ir = jnp.concatenate([jnp.where(row8 == 0, 0.0, ir[:8]), ir[8:]], axis=0)
            ii = jnp.concatenate([jnp.where(row8 == 0, 0.0, ii[:8]), ii[8:]], axis=0)
          xs[0, t * 128:(t + 1) * 128, dcol(a)] = rr - ii
          xs[1, t * 128:(t + 1) * 128, dcol(a)] = ri + ir
      return 0

    lax.fori_loop(0, 4, fwd, 0)

  start(c_w[4:8])
  with jax.named_scope("b_w"):
    wait(c_wt)

    def wperm(ap, _):
      cols = pl.ds(pl.multiple_of(ap * 1024, 1024), 1024)
      for i in range(2):
        for tile in range(4):
          p = _dot(pm[...], wt[i, tile * 128:(tile + 1) * 128, cols]) * (2.0 / (S * D))
          for r in range(8):
            pr = p[16 * r:16 * r + 16]
            if tile == 0 and r == 0:
              first = lax.broadcasted_iota(jnp.int32, (16, 1024), 0) == 0
              pr = jnp.where(first, pr * 0.5, pr)
            r0 = _spectrum_row_of_residue(r) + 16 * tile
            wf[i, r0:r0 + 16, cols] = pr
        ny = wt[i, 512:513, cols].astype(f32) * (1.0 / (S * D))
        wf[i, 512:KR, cols] = jnp.broadcast_to(ny, (8, 1024))
      return 0

    lax.fori_loop(0, 2, wperm, 0, unroll=False)

  with jax.named_scope("b_mid"):
    def mid(i):
      rows = pl.ds(pl.multiple_of(i * 8, 8), 8)
      y = _dft16([(xs[0, rows, col(a)], xs[1, rows, col(a)]) for a in range(16)], -1)
      z = []
      for c in range(16):
        wr, wi = wf[0, rows, col(c)], wf[1, rows, col(c)]
        yr, yi = y[c]
        z.append((yr * wr - yi * wi, yr * wi + yi * wr))
      q = _dft16(z, 1)
      for a in range(16):
        xs[0, rows, col(a)] = q[a][0]
        xs[1, rows, col(a)] = q[a][1]

    def mid_and_q(hp, _):
      at_step(hp, {3: lambda: wait(c_w[1]), 7: lambda: wait(c_w[2] + c_w[3])})
      for u in range(8):
        par, n = u // 4, u % 4
        xv = xq[16 * n:16 * n + 16].reshape(16 * PRE, D)
        qp[2 * hp + par, 16 * n * PRE:(16 * n + 16) * PRE] = _rnd(
            _dot(xv, pltpu.bitcast(wqkv[0, par, hp], bf16)))
        mid(8 * hp + u)
      merge(0, hp + 1)
      return 0

    mid(KR // 8 - 1)
    wait(c_xq + c_w[0])
    merge(0, 0)
    lax.fori_loop(0, 8, mid_and_q, 0)

  start(c_w[8:12] + [c_a0] + c_wo)
  bo_u = out_h.bitcast(u32)
  c_ob = [pltpu.make_async_copy(bx.at[a], bo_u.at[:, a, D:2 * D], sem_out.at[0])
          for a in range(8)]

  with jax.named_scope("b_inv"):
    lane = lax.broadcasted_iota(jnp.int32, (128, 128), 1)

    def inv(ap):
      ys = []
      for par in range(2):
        a = 2 * ap + par
        g = gs[a]
        rs = [_dot_nt(g, jnp.concatenate(
            [xs[0, t * 128:(t + 1) * 128, dcol(a)], xs[1, t * 128:(t + 1) * 128, dcol(a)]],
            axis=0).astype(bf16)) for t in range(4)]
        qn = jnp.concatenate([xs[0, 512:KR, dcol(a)], xs[1, 512:KR, dcol(a)]], axis=1)
        qn = jnp.concatenate([qn, jnp.zeros((120, 256), f32)], axis=0).astype(bf16)
        ny = _dot_nt(jnp.concatenate([g[:128], g[128:]], axis=1), qn)
        z = []
        for t in range(4):
          r = rs[t]
          ur = r[:128, :128] + r[128:, 128:]
          ui = r[:128, 128:] - r[128:, :128]
          if t == 0:
            ui = jnp.where(lane == 0, ny, ui)
          y = _dot(jnp.concatenate([ur, ui], axis=1).astype(bf16), md[t])
          z.append((y[:, :128], y[:, 128:]))
        (z0, z4), (p1, q1), (p2, q2), (p3, q3) = z
        ep, op = z0 + z4, z0 - z4
        e0, e2, o0, o2 = ep + p2, ep - p2, op + q2, op - q2
        e1, e3 = p1 + p3, q1 - q3
        u, v = (p1 - p3) * rc, (q1 + q3) * rc
        o1, o3 = v + u, v - u
        ys.append([e0 + e1, o0 + o1, e2 + e3, o2 + o3, e0 - e1, o0 - o1, e2 - e3, o2 - o3])
      for j in range(8):
        lo = pltpu.bitcast(_rnd(ys[0][j]), u32)
        hi = pltpu.bitcast(_rnd(ys[1][j]), u32)
        bx[ap, :, col(j)] = (lo >> 16) | hi

    def inv2(it, _):
      inv(2 * it)
      inv(2 * it + 1)
      return 0

    lax.fori_loop(0, 4, inv2, 0)


  def w1(m, h):
    return pltpu.bitcast(wqkv[m, h % 2, h // 2], bf16)

  def w2(j, g):
    return pltpu.bitcast(wo[j, g * G * 64:(g + 1) * G * 64], bf16)

  with jax.named_scope("q_pre"):
    def q_pre(it, _):
      for u in range(4):
        project(0, 8 + 4 * it + u, qp)
        if u < 3:
          merge(0, 9 + 4 * it + u)
        merge(1, 8 * it + 2 * u)
        merge(1, 8 * it + 2 * u + 1)
      return 0

    wait(c_w[4] + c_w[5] + c_w[6] + c_w[7])
    merge(0, 12)
    lax.fori_loop(0, 2, q_pre, 0)

  with jax.named_scope("k_pre"):
    wait(c_w[8] + c_w[9] + c_w[10] + c_w[11])
    for u in range(KPRE // 2):
      project(1, u, kp)
      for n in range(32 // KPRE):
        merge(2, 32 // KPRE * u + n)

  row = lax.broadcasted_iota(jnp.int32, (L, L), 0)
  colm = lax.broadcasted_iota(jnp.int32, (L, L), 1)
  mask = (row < M) | (row >= colm)
  scale = DH ** -0.5

  def out_copy(c):
    n = OUT_CHUNK * SEG // 16
    rows = pl.ds(c * n, n)
    return pltpu.make_async_copy(ao.at[rows], out_h.at[rows, :, 0:D], sem_out.at[1])

  order = []
  for g in range(NG):
    order += [("qk", g)] + ([("pv", g - 1)] if g >= 1 else [])
    order += [("v", g), ("sc", g)] + ([("wo", g - 2)] if g >= 2 else [])
  order += [("pv", NG - 1), ("wo", NG - 2), ("wo", NG - 1)]

  def step(s, mem):
    hl = jnp.concatenate([mem, ax[s].astype(f32)], axis=0)
    pre = pl.ds(pl.multiple_of(s * PRE, PRE), PRE)
    q, k, v, p, o = {}, {}, {}, {}, {}
    y = [None] * 8
    for op, g in order:
      hs = range(g * G, (g + 1) * G)
      for h in hs:
        if op == "qk":
          q[h] = jnp.concatenate([_rnd(_dot(hl[:L - PRE], w1(0, h))), qp[h, pre, :]], axis=0)
          if h < KPRE:
            k[h] = jnp.concatenate([_dot(hl[:L - PRE], w1(1, h)), kp[h, pre, :]], axis=0).astype(bf16)
          else:
            k[h] = _dot(hl, w1(1, h)).astype(bf16)
        elif op == "v":
          v[h] = _dot(hl, w1(2, h)).astype(bf16)
        elif op == "sc":
          sc = jnp.where(mask, _dot_nt(q[h], k[h]) * scale, -1e9)
          e = jnp.exp(sc - jnp.max(sc, axis=-1, keepdims=True))
          p[h] = _rnd(e / jnp.sum(e, axis=-1, keepdims=True))
        elif op == "pv":
          o[h] = _rnd(_dot(p[h], v[h]))
      if op == "wo":
        og = jnp.concatenate([o[h] for h in hs], axis=1)
        for j in range(8):
          t = _dot(og, w2(j, g))
          y[j] = t if y[j] is None else y[j] + t
    yb = jnp.concatenate(y, axis=1).astype(bf16)
    ao[pl.ds(2 * s, 2)] = yb[M:].reshape(2, 16, D)
    return yb[:M].astype(f32)

  with jax.named_scope("a_wait"):
    wait(c_a0 + c_wo[0] + c_wo[1])
  start([c_a1, c_ob])

  def steps(i, mem):
    s = UNROLL * i

    @pl.when(s == OUT_CHUNK)
    def _():
      wait(c_a1)

    for u in range(UNROLL):
      mem = step(s + u, mem)

    @pl.when((s + UNROLL) % OUT_CHUNK == 0)
    def _():
      out_copy(s // OUT_CHUNK).start()

    return mem

  with jax.named_scope("a_loop"):
    lax.fori_loop(0, NSEG // UNROLL, steps, mem0[...].astype(f32))

  with jax.named_scope("wait_out"):
    wait(c_ob)
    for c in range(NSEG // OUT_CHUNK):
      out_copy(c).wait()


@functools.partial(jax.jit, static_argnames=("A_seg_len",))
def pallas_concat_heads__memory_aug_recurrent_mem_tr__spectral_gfnet__prompt_kernel(
    A_x, A_mem0, A_Wq, A_Wk, A_Wv, A_Wo, A_seg_len, B_x, B_w_r, B_w_i):
  assert A_seg_len == SEG and A_x.shape == (1, S, D) and A_Wq.shape == (D, H, DH)
  consts = _constants()
  hbm = pl.BlockSpec(memory_space=pltpu.HBM)
  out = pl.pallas_call(
      _kernel,
      out_shape=jax.ShapeDtypeStruct((S // 16, 16, 2 * D), bf16),
      in_specs=[hbm] * 12,
      out_specs=hbm,
      scratch_shapes=[
          pltpu.VMEM((3, 2, H // 2, D // 2, DH), u32),
          pltpu.VMEM((D // 128, H * DH // 2, 128), u32),
          pltpu.VMEM((NSEG, SEG, D), bf16),
          pltpu.VMEM((M, D), bf16),
          pltpu.VMEM((8, 128, D), u32),
          pltpu.VMEM((2, D // 2 + 1, S), bf16),
          pltpu.VMEM((4, 256, 256), bf16),
          pltpu.VMEM((128, 128), bf16),
          pltpu.VMEM((16, 256, 128), bf16),
          pltpu.VMEM((2, KR, S), f32),
          pltpu.VMEM((2, KR, S), f32),
          pltpu.VMEM((S // 16, 16, D), bf16),
          pltpu.VMEM((NSEG, PRE, D), bf16),
          pltpu.VMEM((H, NSEG * PRE, DH), f32),
          pltpu.VMEM((KPRE, NSEG * PRE, DH), f32),
          pltpu.SemaphoreType.DMA((64,)),
          pltpu.SemaphoreType.DMA((2,)),
      ],
      compiler_params=pltpu.CompilerParams(vmem_limit_bytes=110 * 2**20),
  )(A_x.reshape(NSEG, SEG, D), A_mem0.reshape(M, D),
    A_Wq.reshape(D // 2, 2, H, DH), A_Wk.reshape(D // 2, 2, H, DH), A_Wv.reshape(D // 2, 2, H, DH),
    A_Wo.reshape(H * DH, D), B_x.reshape(S // 16, 16, D),
    B_w_r.T, B_w_i.T, *consts)
  return out.reshape(1, S, 2 * D)
```

```python
import functools

import jax
import jax.numpy as jnp
import numpy as np
from jax import lax
import jax.experimental.pallas as pl
import jax.experimental.pallas.tpu as pltpu

f32, bf16, u32 = jnp.float32, jnp.bfloat16, jnp.uint32

S, D = 2048, 1024
H, DH = 32, 128
M, SEG = 8, 32
L = M + SEG
NSEG = S // SEG
X_HEAD = 8
G = 4
NG = H // G
PRE = 8
KPRE = 8
UNROLL = 2
KR = D // 2 + 8


def _kd_of_row():
  kd = np.zeros(512, np.int64)
  l = np.arange(64)
  for t in range(4):
    kd[128 * t:128 * t + 64] = t + 8 * l
    kd[128 * t + 64:128 * t + 128] = (8 - t if t else 4) + 8 * l
  return kd


def _spectrum_row_of_residue(r):
  if r < 4:
    return 128 * r
  return 64 if r == 4 else 128 * (8 - r) + 64


def _constants():
  kd = _kd_of_row()
  b = np.arange(128)
  lo = (b < 64)[:, None]
  md = np.zeros((4, 256, 256))
  for t in range(4):
    e = np.exp(-2j * np.pi * np.outer(kd[128 * t:128 * t + 128], b) / D)
    c, s = e.real, e.imag
    if t == 0:
      md[0, :128, :128], md[0, 128:, :128] = np.where(lo, c, 0), np.where(lo, s, 0)
      md[0, :128, 128:], md[0, 128:, 128:] = np.where(lo, 0, c), np.where(lo, 0, s)
      md[0, 128, :128] = (-1.0) ** b
    else:
      sg = np.where(lo, 1.0, -1.0)
      md[t, :128, :128], md[t, 128:, :128] = c, s
      md[t, :128, 128:], md[t, 128:, 128:] = sg * s, -sg * c
  pm = np.zeros((128, 128))
  pm[b, b // 16 + 8 * (b % 16)] = 1.0
  gs = np.zeros((16, 256, 128))
  for a in range(16):
    g = np.exp(-2j * np.pi * np.outer(a + 16 * b, b) / S)
    gs[a, :128], gs[a, 128:] = g.real, g.imag
  cast = lambda a: a.astype(np.float32).astype(jnp.bfloat16)
  return cast(md), cast(pm), cast(gs)


def _dft4(z, sign):
  (ar, ai), (br, bi), (cr, ci), (dr, di) = z
  t0r, t0i, t1r, t1i = ar + cr, ai + ci, ar - cr, ai - ci
  t2r, t2i, t3r, t3i = br + dr, bi + di, br - dr, bi - di
  p = (t1r + t3i, t1i - t3r)
  m = (t1r - t3i, t1i + t3r)
  x1, x3 = (p, m) if sign < 0 else (m, p)
  return [(t0r + t2r, t0i + t2i), x1, (t0r - t2r, t0i - t2i), x3]


def _cmul_w16(z, n, sign):
  zr, zi = z
  if n == 0:
    return z
  if n == 4:
    return (zi, -zr) if sign < 0 else (-zi, zr)
  c = float(np.cos(2 * np.pi * n / 16))
  s = float(sign * np.sin(2 * np.pi * n / 16))
  if n == 2:
    return ((zr + zi) * c, (zi - zr) * c) if sign < 0 else ((zr - zi) * c, (zi + zr) * c)
  if n == 6:
    h = -c
    return ((zi - zr) * h, (zr + zi) * -h) if sign < 0 else ((zr + zi) * -h, (zr - zi) * h)
  return (zr * c - zi * s, zr * s + zi * c)


def _dft16(x, sign):
  t = [_dft4([x[a2], x[4 + a2], x[8 + a2], x[12 + a2]], sign) for a2 in range(4)]
  out = [None] * 16
  for k1 in range(4):
    r = _dft4([_cmul_w16(t[a2][k1], a2 * k1, sign) for a2 in range(4)], sign)
    for k2 in range(4):
      out[k1 + 4 * k2] = r[k2]
  return out


def _rnd(a):
  return a.astype(bf16).astype(f32)


def _dot(a, b):
  return jnp.dot(a, b, preferred_element_type=f32)


def _dot_nt(a, b):
  return lax.dot_general(a, b, (((1,), (1,)), ((), ())), preferred_element_type=f32)


def _kernel(ax_h, mem_h, wq_h, wk_h, wv_h, wo_h, bx_h, wr_h, wi_h, md_h, pm_h, gs_h, out_h,
            wqkv, wo, ax, mem0, bx, wt, md, pm, gs, xs, wf, ao, xq, qp, kp, sem_in, sem_out):
  nsem = [0]

  def group(pairs):
    i = nsem[0]
    nsem[0] += 1
    return [pltpu.make_async_copy(s, d, sem_in.at[i]) for s, d in pairs]

  def wait(copies):
    for c in copies:
      c.wait()

  bx_u = bx_h.bitcast(u32)
  c_const = group([(md_h, md)])
  c_bx = [group([(bx_u.at[:, a, :], bx.at[a]), (gs_h.at[2 * a:2 * a + 2], gs.at[2 * a:2 * a + 2])])
          for a in range(8)]
  c_wt = group([(wr_h, wt.at[0]), (pm_h, pm), (wi_h, wt.at[1])])
  w_u = [w_h.bitcast(u32) for w_h in (wq_h, wk_h, wv_h)]
  wo_u = wo_h.bitcast(u32)

  def w_group(m, g):
    return group([(w_u[m].at[:, par, hp, :], wqkv.at[m, par, hp])
                  for hp in range(4 * g, 4 * g + 4) for par in range(2)])

  c_w = [w_group(m, g) for m in range(3) for g in range(4)]
  c_wo = [group([(wo_u.at[i * 1024:(i + 1) * 1024, j * 128:(j + 1) * 128],
                  wo.at[j, i * 1024:(i + 1) * 1024]) for j in range(8)]) for i in range(2)]
  c_xq = group([(ax_h.at[:, SEG - PRE:SEG, :], xq)])
  c_a0 = group([(mem_h, mem0), (ax_h.at[0:X_HEAD], ax.at[0:X_HEAD])])
  c_a1 = group([(ax_h.at[X_HEAD:NSEG], ax.at[X_HEAD:NSEG])])

  def start(groups):
    for g in groups:
      for c in g:
        c.start()

  with jax.named_scope("dma_start"):
    start([c_const])
    start(c_bx + [c_wt, c_xq] + c_w[0:4])

  def at_step(i, table):
    for n, fn in table.items():
      pl.when(i == n)(fn)

  def merge(m, hp):
    for r in range(4):
      rows = pl.ds(r * 128, 128)
      a, b = wqkv[m, 0, hp, rows, :], wqkv[m, 1, hp, rows, :]
      wqkv[m, 0, hp, rows, :] = (a & 0xFFFF) | (b << 16)
      wqkv[m, 1, hp, rows, :] = (a >> 16) | (b & jnp.uint32(0xFFFF0000))

  def project(m, hp, dst):
    xv = xq[...].reshape(NSEG * PRE, D)
    for par in range(2):
      dst[2 * hp + par] = _rnd(_dot(xv, pltpu.bitcast(wqkv[m, par, hp], bf16)))

  rc = float(np.sqrt(0.5))

  def col(c):
    return pl.ds(c * 128, 128)

  def dcol(c):
    return pl.ds(pl.multiple_of(c * 128, 128), 128)

  with jax.named_scope("b_fwd"):
    wait(c_const)
    row8 = lax.broadcasted_iota(jnp.int32, (8, 128), 0)

    def fwd(it, _):
      at_step(it, {n: functools.partial(wait, c_bx[2 * n] + c_bx[2 * n + 1]) for n in range(4)})
      for u in range(4):
        a, ap, par = 4 * it + u, 2 * it + u // 2, u % 2
        w = [bx[ap, :, col(j)] for j in range(8)]
        x = [pltpu.bitcast(v << 16 if par == 0 else v & jnp.uint32(0xFFFF0000), f32) for v in w]
        e0, e1, e2, e3 = x[0] + x[4], x[0] - x[4], x[2] + x[6], x[2] - x[6]
        o0, o1, o2, o3 = x[1] + x[5], x[1] - x[5], x[3] + x[7], x[3] - x[7]
        ep, op = e0 + e2, o0 + o2
        u, v = (o1 - o3) * rc, (o1 + o3) * rc
        z = [(ep + op, ep - op), (e1 + u, v + e3), (e0 - e2, o0 - o2), (e1 - u, v - e3)]
        tt = [_dot_nt(md[t], jnp.concatenate(z[t], axis=1).astype(bf16)) for t in range(4)]
        g = jnp.concatenate([gs[a, :128], gs[a, 128:]], axis=1)
        for t in range(4):
          r = _dot(tt[t].astype(bf16), g)
          rr, ri, ir, ii = r[:128, :128], r[:128, 128:], r[128:, :128], r[128:, 128:]
          if t == 0:
            xs[0, 512:KR, dcol(a)] = jnp.where(row8 == 0, ir[:8], 0.0)
            xs[1, 512:KR, dcol(a)] = jnp.where(row8 == 0, ii[:8], 0.0)
            ir = jnp.concatenate([jnp.where(row8 == 0, 0.0, ir[:8]), ir[8:]], axis=0)
            ii = jnp.concatenate([jnp.where(row8 == 0, 0.0, ii[:8]), ii[8:]], axis=0)
          xs[0, t * 128:(t + 1) * 128, dcol(a)] = rr - ii
          xs[1, t * 128:(t + 1) * 128, dcol(a)] = ri + ir
      return 0

    lax.fori_loop(0, 4, fwd, 0)

  start(c_w[4:8])
  with jax.named_scope("b_w"):
    wait(c_wt)

    def wperm(ap, _):
      cols = pl.ds(pl.multiple_of(ap * 1024, 1024), 1024)
      for i in range(2):
        for tile in range(4):
          p = _dot(pm[...], wt[i, tile * 128:(tile + 1) * 128, cols]) * (2.0 / (S * D))
          for r in range(8):
            pr = p[16 * r:16 * r + 16]
            if tile == 0 and r == 0:
              first = lax.broadcasted_iota(jnp.int32, (16, 1024), 0) == 0
              pr = jnp.where(first, pr * 0.5, pr)
            r0 = _spectrum_row_of_residue(r) + 16 * tile
            wf[i, r0:r0 + 16, cols] = pr
        ny = wt[i, 512:513, cols].astype(f32) * (1.0 / (S * D))
        wf[i, 512:KR, cols] = jnp.broadcast_to(ny, (8, 1024))
      return 0

    lax.fori_loop(0, 2, wperm, 0, unroll=False)

  with jax.named_scope("b_mid"):
    def mid(i):
      rows = pl.ds(pl.multiple_of(i * 8, 8), 8)
      y = _dft16([(xs[0, rows, col(a)], xs[1, rows, col(a)]) for a in range(16)], -1)
      z = []
      for c in range(16):
        wr, wi = wf[0, rows, col(c)], wf[1, rows, col(c)]
        yr, yi = y[c]
        z.append((yr * wr - yi * wi, yr * wi + yi * wr))
      q = _dft16(z, 1)
      for a in range(16):
        xs[0, rows, col(a)] = q[a][0]
        xs[1, rows, col(a)] = q[a][1]

    def mid_and_q(it, _):
      at_step(it, {1: lambda: wait(c_w[1]), 3: lambda: wait(c_w[2]),
                   4: lambda: start(c_w[8:12] + [c_a0] + c_wo),
                   5: lambda: wait(c_w[3]), 7: lambda: wait(c_w[4])})
      for hh in range(2):
        hp = 2 * it + hh
        for u in range(4):
          par, n = u // 2, u % 2
          xv = xq[32 * n:32 * n + 32].reshape(32 * PRE, D)
          qp[2 * hp + par, 32 * n * PRE:(32 * n + 32) * PRE] = _rnd(
              _dot(xv, pltpu.bitcast(wqkv[0, par, hp], bf16)))
          mid(4 * hp + u)
        merge((hp + 2) // 16, (hp + 2) % 16)
      return 0

    mid(KR // 8 - 1)
    wait(c_xq + c_w[0])
    for hp in range(2):
      merge(0, hp)
    lax.fori_loop(0, H // 4, mid_and_q, 0)

  bo_u = out_h.bitcast(u32)
  c_ob = [pltpu.make_async_copy(bx.at[a], bo_u.at[:, a, D:2 * D], sem_out.at[0])
          for a in range(8)]

  with jax.named_scope("b_inv"):
    lane = lax.broadcasted_iota(jnp.int32, (128, 128), 1)

    def inv(ap):
      ys = []
      for par in range(2):
        a = 2 * ap + par
        g = gs[a]
        rs = [_dot_nt(g, jnp.concatenate(
            [xs[0, t * 128:(t + 1) * 128, dcol(a)], xs[1, t * 128:(t + 1) * 128, dcol(a)]],
            axis=0).astype(bf16)) for t in range(4)]
        qn = jnp.concatenate([xs[0, 512:KR, dcol(a)], xs[1, 512:KR, dcol(a)]], axis=1)
        qn = jnp.concatenate([qn, jnp.zeros((120, 256), f32)], axis=0).astype(bf16)
        ny = _dot_nt(jnp.concatenate([g[:128], g[128:]], axis=1), qn)
        z = []
        for t in range(4):
          r = rs[t]
          ur = r[:128, :128] + r[128:, 128:]
          ui = r[:128, 128:] - r[128:, :128]
          if t == 0:
            ui = jnp.where(lane == 0, ny, ui)
          y = _dot(jnp.concatenate([ur, ui], axis=1).astype(bf16), md[t])
          z.append((y[:, :128], y[:, 128:]))
        (z0, z4), (p1, q1), (p2, q2), (p3, q3) = z
        ep, op = z0 + z4, z0 - z4
        e0, e2, o0, o2 = ep + p2, ep - p2, op + q2, op - q2
        e1, e3 = p1 + p3, q1 - q3
        u, v = (p1 - p3) * rc, (q1 + q3) * rc
        o1, o3 = v + u, v - u
        ys.append([e0 + e1, o0 + o1, e2 + e3, o2 + o3, e0 - e1, o0 - o1, e2 - e3, o2 - o3])
      for j in range(8):
        lo = pltpu.bitcast(_rnd(ys[0][j]), u32)
        hi = pltpu.bitcast(_rnd(ys[1][j]), u32)
        bx[ap, :, col(j)] = (lo >> 16) | hi

    def inv2(it, _):
      for u in range(2):
        inv(2 * it + u)
        for n in range(2 - u):
          merge(1, 2 + 3 * it + 2 * u + n)
      return 0

    wait(c_w[5] + c_w[6] + c_w[7])
    lax.fori_loop(0, 4, inv2, 0)


  def w1(m, h):
    return pltpu.bitcast(wqkv[m, h % 2, h // 2], bf16)

  def w2(j, g):
    return pltpu.bitcast(wo[j, g * G * 64:(g + 1) * G * 64], bf16)

  with jax.named_scope("k_pre"):
    wait(c_w[8] + c_w[9] + c_w[10] + c_w[11])
    for u in range(KPRE // 2):
      for n in (2 * u, 2 * u + 1):
        kp[n] = _rnd(_dot(xq[...].reshape(NSEG * PRE, D), w1(1, G * n)))
      for n in range(32 // KPRE):
        merge(2, 32 // KPRE * u + n)
      if u < 2:
        merge(1, 14 + u)

  row = lax.broadcasted_iota(jnp.int32, (L, L), 0)
  colm = lax.broadcasted_iota(jnp.int32, (L, L), 1)
  mask = (row < M) | (row >= colm)
  scale = DH ** -0.5

  def out_copy(c):
    n = UNROLL * SEG // 16
    rows = pl.ds(c * n, n)
    return pltpu.make_async_copy(ao.at[rows], out_h.at[rows, :, 0:D], sem_out.at[1])

  order = []
  for g in range(NG):
    order += [("qk", g)] + ([("pv", g - 1)] if g >= 1 else [])
    order += [("v", g), ("sc", g)] + ([("wo", g - 2)] if g >= 2 else [])
  order += [("pv", NG - 1), ("wo", NG - 2), ("wo", NG - 1)]

  def step(s, mem):
    hl = jnp.concatenate([mem, ax[s].astype(f32)], axis=0)
    pre = pl.ds(pl.multiple_of(s * PRE, PRE), PRE)
    q, k, v, p, o = {}, {}, {}, {}, {}
    y = [None] * 8
    for op, g in order:
      hs = range(g * G, (g + 1) * G)
      for h in hs:
        if op == "qk":
          q[h] = jnp.concatenate([_rnd(_dot(hl[:L - PRE], w1(0, h))), qp[h, pre, :]], axis=0)
          if h % G == 0:
            k[h] = jnp.concatenate([_dot(hl[:L - PRE], w1(1, h)), kp[h // G, pre, :]], axis=0).astype(bf16)
          else:
            k[h] = _dot(hl, w1(1, h)).astype(bf16)
        elif op == "v":
          v[h] = _dot(hl, w1(2, h)).astype(bf16)
        elif op == "sc":
          sc = jnp.where(mask, _dot_nt(q[h], k[h]) * scale, -1e9)
          e = jnp.exp(sc - jnp.max(sc, axis=-1, keepdims=True))
          p[h] = _rnd(e / jnp.sum(e, axis=-1, keepdims=True))
        elif op == "pv":
          o[h] = _rnd(_dot(p[h], v[h]))
      if op == "wo":
        og = jnp.concatenate([o[h] for h in hs], axis=1)
        for j in range(8):
          t = _dot(og, w2(j, g))
          y[j] = t if y[j] is None else y[j] + t
    yb = jnp.concatenate(y, axis=1).astype(bf16)
    ao[pl.ds(2 * s, 2)] = yb[M:].reshape(2, 16, D)
    return yb[:M].astype(f32)

  with jax.named_scope("a_wait"):
    wait(c_a0 + c_wo[0] + c_wo[1])
  start([c_ob, c_a1])

  def steps(i, mem):
    s = UNROLL * i

    @pl.when(s == X_HEAD)
    def _():
      wait(c_a1)

    for u in range(UNROLL):
      mem = step(s + u, mem)
    at_step(i, {0: lambda: wait(c_ob)})
    out_copy(i).start()
    return mem

  with jax.named_scope("a_loop"):
    lax.fori_loop(0, NSEG // UNROLL, steps, mem0[...].astype(f32))

  with jax.named_scope("wait_out"):
    for c in range(NSEG // UNROLL):
      out_copy(c).wait()


@functools.partial(jax.jit, static_argnames=("A_seg_len",))
def pallas_concat_heads__memory_aug_recurrent_mem_tr__spectral_gfnet__prompt_kernel(
    A_x, A_mem0, A_Wq, A_Wk, A_Wv, A_Wo, A_seg_len, B_x, B_w_r, B_w_i):
  assert A_seg_len == SEG and A_x.shape == (1, S, D) and A_Wq.shape == (D, H, DH)
  consts = _constants()
  hbm = pl.BlockSpec(memory_space=pltpu.HBM)
  out = pl.pallas_call(
      _kernel,
      out_shape=jax.ShapeDtypeStruct((S // 16, 16, 2 * D), bf16),
      in_specs=[hbm] * 12,
      out_specs=hbm,
      scratch_shapes=[
          pltpu.VMEM((3, 2, H // 2, D // 2, DH), u32),
          pltpu.VMEM((D // 128, H * DH // 2, 128), u32),
          pltpu.VMEM((NSEG, SEG, D), bf16),
          pltpu.VMEM((M, D), bf16),
          pltpu.VMEM((8, 128, D), u32),
          pltpu.VMEM((2, D // 2 + 1, S), bf16),
          pltpu.VMEM((4, 256, 256), bf16),
          pltpu.VMEM((128, 128), bf16),
          pltpu.VMEM((16, 256, 128), bf16),
          pltpu.VMEM((2, KR, S), f32),
          pltpu.VMEM((2, KR, S), f32),
          pltpu.VMEM((S // 16, 16, D), bf16),
          pltpu.VMEM((NSEG, PRE, D), bf16),
          pltpu.VMEM((H, NSEG * PRE, DH), f32),
          pltpu.VMEM((KPRE, NSEG * PRE, DH), f32),
          pltpu.SemaphoreType.DMA((64,)),
          pltpu.SemaphoreType.DMA((2,)),
      ],
      compiler_params=pltpu.CompilerParams(vmem_limit_bytes=110 * 2**20),
  )(A_x.reshape(NSEG, SEG, D), A_mem0.reshape(M, D),
    A_Wq.reshape(D // 2, 2, H, DH), A_Wk.reshape(D // 2, 2, H, DH), A_Wv.reshape(D // 2, 2, H, DH),
    A_Wo.reshape(H * DH, D), B_x.reshape(S // 16, 16, D),
    B_w_r.T, B_w_i.T, *consts)
  return out.reshape(1, S, 2 * D)
```
